```python
import jax
import jax.numpy as jnp

def _softmax(x, axis=-1):
    return jax.nn.softmax(x, axis=axis)
def _gelu(x):
    return jax.nn.gelu(x, approximate=True)
def _silu(x):
    return jax.nn.silu(x)
def _sigmoid(x):
    return jax.nn.sigmoid(x)
def _layernorm(x, axis=-1, eps=1e-5):
    m = jnp.mean(x, axis=axis, keepdims=True)
    v = jnp.var(x, axis=axis, keepdims=True)
    return (x - m) / jnp.sqrt(v + eps)
def _scatter_add(tgt, idx, src, axis=0):
    return tgt.at[idx].add(src)
def _segment_sum(src, seg, n):
    return jax.ops.segment_sum(src, seg, n)
class _Rng:
    def __init__(self, key):
        self._k = key
    def _next(self):
        self._k, sub = jax.random.split(self._k)
        return sub
    def normal(self, shape):
        return jax.random.normal(self._next(), shape, dtype=jnp.bfloat16)
    def randint(self, lo, hi, shape):
        return jax.random.randint(self._next(), shape, lo, hi, dtype=jnp.int32)
    def uniform(self, shape, lo=0.0, hi=1.0):
        return jax.random.uniform(self._next(), shape, jnp.bfloat16, lo, hi)
    def permutation(self, n):
        return jax.random.permutation(self._next(), n)


kernel_name = 'concat_heads__spectral_gfnet__compressed_kv_cla__prompt'

def setup_inputs():
    _rng = _Rng(jax.random.key(int.from_bytes(__import__("os").urandom(4), "little")))
    _w = (lambda a: (lambda t: t.astype(jnp.bfloat16) if jnp.issubdtype(t.dtype, jnp.floating) else t)(jnp.asarray(a)))
    def _A_setup():
        B, S, D = 1, 2048, 448
        Df = D // 2 + 1
        return {
            "x": _w((lambda *s: _rng.normal(s) * 0.05)(B, S, D)),
            "w_r": _w((lambda *s: _rng.normal(s) * 0.05)(S, Df) * 0.02),
            "w_i": _w((lambda *s: _rng.normal(s) * 0.05)(S, Df) * 0.02),
        }
    _A_in = _A_setup()

    def _B_setup():
        B, H, Sq, Sk, D, M = 1, 16, 2048, 2048, 256, 448
        Dc = 4 * D
        return {
            "x": _w((lambda *s: _rng.normal(s) * 0.05)(B, Sq, M)),
            "c_kv": _w((lambda *s: _rng.normal(s) * 0.05)(B, Sk, Dc)),
            "w_q": _w((lambda *s: _rng.normal(s) * 0.05)(M, H, D) * (M ** -0.5)),
            "w_uk": _w((lambda *s: _rng.normal(s) * 0.05)(Dc, H, D) * (Dc ** -0.5)),
            "w_uv": _w((lambda *s: _rng.normal(s) * 0.05)(Dc, H, D) * (Dc ** -0.5)),
            "w_o": _w((lambda *s: _rng.normal(s) * 0.05)(H, D, M) * ((H * D) ** -0.5)),
        }
    _B_in = _B_setup()

    return {
        "A_x": _A_in["x"],
        "A_w_r": _A_in["w_r"],
        "A_w_i": _A_in["w_i"],
        "B_x": _B_in["x"],
        "B_c_kv": _B_in["c_kv"],
        "B_w_q": _B_in["w_q"],
        "B_w_uk": _B_in["w_uk"],
        "B_w_uv": _B_in["w_uv"],
        "B_w_o": _B_in["w_o"],
    }

def reference(A_x, A_w_r, A_w_i, B_x, B_c_kv, B_w_q, B_w_uk, B_w_uv, B_w_o):
    def _A_ref(x, w_r, w_i):
        B, S, D = x.shape
        X = (lambda x, axes=(-2,-1): jnp.fft.rfft2(x.astype(jnp.float32), axes=axes))(x, axes=(-2, -1))
        W = w_r + 1j * w_i
        X = X * W
        y = (lambda x, s, axes=(-2,-1): jnp.fft.irfft2(x, s=s, axes=axes).astype(jnp.bfloat16))(X, (S, D), axes=(-2, -1))
        return y

    def _B_ref(x, c_kv, w_q, w_uk, w_uv, w_o):
        B, Sq, M = x.shape[0], x.shape[1], x.shape[2]
        Sk = c_kv.shape[1]
        H, D = w_q.shape[1], w_q.shape[2]
        q = jnp.einsum("bqm,mhd->bhqd", x, w_q)
        k = jnp.einsum("bkc,chd->bhkd", c_kv, w_uk)
        v = jnp.einsum("bkc,chd->bhkd", c_kv, w_uv)
        scores = jnp.einsum("bhqd,bhkd->bhqk", q, k) * (D ** -0.5)
        off = Sk - Sq
        qi = jnp.arange(Sq)[:, None]
        kj = jnp.arange(Sk)[None, :]
        cmask = kj <= (qi + off)
        scores = jnp.where(cmask[None, None], scores, -1e9)
        p = _softmax(scores, axis=-1)
        ctx = jnp.einsum("bhqk,bhkd->bhqd", p, v)
        return jnp.einsum("bhqd,hdm->bqm", ctx, w_o)

    a = _A_ref(A_x, A_w_r, A_w_i)
    b = _B_ref(B_x, B_c_kv, B_w_q, B_w_uk, B_w_uv, B_w_o)
    return jnp.concatenate([a, b], axis=-1)
```

```python
import functools

import jax
import jax.numpy as jnp
import numpy as np
from jax import lax
import jax.experimental.pallas as pl
import jax.experimental.pallas.tpu as pltpu

_BF16 = jnp.bfloat16
_F32 = jnp.float32
_NT = (((1,), (1,)), ((), ()))
_LOG2E = 1.4426950408889634
_NEG = -1e30


def _np_bf16(a):
    import ml_dtypes
    return np.asarray(a, np.float64).astype(np.float32).astype(ml_dtypes.bfloat16)


@functools.lru_cache(maxsize=None)
def _dft_tables(S, D):
    Df = D // 2 + 1
    n1, n2 = 16, S // 16
    d = np.arange(D)[:, None]
    c = np.arange(Df)[None, :]
    ang = 2.0 * np.pi * ((d * c) % D) / D
    fdr = np.cos(ang)
    fdi = -np.sin(ang)
    wgt = np.full(Df, 2.0)
    wgt[0] = 1.0
    if D % 2 == 0:
        wgt[-1] = 1.0
    gdr = wgt[:, None] * np.cos(ang.T) / (S * D)
    gdi = -wgt[:, None] * np.sin(ang.T) / (S * D)
    k1 = np.arange(n1)[:, None, None]
    k2 = np.arange(n2)[None, :, None]
    b = np.arange(n2)[None, None, :]
    g = np.exp(-2j * np.pi * ((b * (k1 + n1 * k2)) % S) / S)
    gf = np.concatenate([g.real, g.imag], axis=1)
    gt = np.transpose(g, (0, 2, 1))
    gi = np.concatenate([gt.real, gt.imag], axis=1)
    return tuple(_np_bf16(t) for t in (fdr, fdi, gf, gi, gdr, gdi))


_R2 = float(np.sqrt(0.5))
_C1, _S1 = float(np.cos(np.pi / 8)), float(np.sin(np.pi / 8))


def _cmul(ar, ai, wr, wi):
    return ar * wr - ai * wi, ar * wi + ai * wr


def _tw16(ar, ai, e, sign):
    e %= 16
    if e == 0:
        return ar, ai
    if e == 4:
        return (-ai, ar) if sign > 0 else (ai, -ar)
    if e == 2:
        return ((ar - ai) * _R2, (ar + ai) * _R2) if sign > 0 else ((ar + ai) * _R2, (ai - ar) * _R2)
    if e == 6:
        return ((-ar - ai) * _R2, (ar - ai) * _R2) if sign > 0 else ((ai - ar) * _R2, (-ar - ai) * _R2)
    ang = sign * 2.0 * np.pi * e / 16
    return _cmul(ar, ai, float(np.cos(ang)), float(np.sin(ang)))


def _dft4(x, sign):
    (ar, ai), (br, bi), (cr, ci), (dr, di) = x
    t0r, t0i = ar + cr, ai + ci
    t1r, t1i = ar - cr, ai - ci
    t2r, t2i = br + dr, bi + di
    t3r, t3i = br - dr, bi - di
    y0 = (t0r + t2r, t0i + t2i)
    y2 = (t0r - t2r, t0i - t2i)
    if sign < 0:
        y1 = (t1r + t3i, t1i - t3r)
        y3 = (t1r - t3i, t1i + t3r)
    else:
        y1 = (t1r - t3i, t1i + t3r)
        y3 = (t1r + t3i, t1i - t3r)
    return [y0, y1, y2, y3]


def _dft16(x, sign):
    cols = []
    for n2 in range(4):
        y = _dft4([x[4 * n1 + n2] for n1 in range(4)], sign)
        cols.append([_tw16(y[k1][0], y[k1][1], n2 * k1, sign) for k1 in range(4)])
    out = [None] * 16
    for k1 in range(4):
        z = _dft4([cols[n2][k1] for n2 in range(4)], sign)
        for k2 in range(4):
            out[k1 + 4 * k2] = z[k2]
    return out


def _dot(a, b):
    return jnp.dot(a, b, preferred_element_type=_F32)


def _dot_nt(a, b):
    return lax.dot_general(a, b, _NT, preferred_element_type=_F32)


def _kernel(ax_h, wr_h, wi_h, bx_h, ckv_h, wq_h, wuk_h, wuv_h, wo_h,
            fdr_h, fdi_h, gf_h, gi_h, gdr_h, gdi_h,
            out_h,
            ax, wr, wi, bx, ckv, wq, wuk, wuv, wo, fdr, fdi, gf, gi, gdr, gdi,
            x1r, x1i, tr, ti, wrp, wip,
            wq_t, wkv_t, q_all, kv, acc, stage, sem, osem,
            *, S, M, H, D, C, BQ):
    Df = M // 2 + 1
    NB = 16
    RB = S // NB
    CCH = 128
    nch = C // CCH

    copies = {}
    sem_ids = {}

    def start(name, src, dst):
        i = len(sem_ids)
        sem_ids[name] = i
        cp = pltpu.make_async_copy(src, dst, sem.at[i])
        cp.start()
        copies[name] = cp

    def wait(*names):
        for n in names:
            copies[n].wait()

    start("ax", ax_h.at[0], ax)
    start("fdr", fdr_h, fdr)
    start("fdi", fdi_h, fdi)
    start("gf", gf_h, gf)
    start("wr", wr_h, wr)
    start("wi", wi_h, wi)
    start("gi", gi_h, gi)
    start("gdr", gdr_h, gdr)
    start("gdi", gdi_h, gdi)
    start("wq", wq_h, wq)
    start("bx", bx_h.at[0], bx)
    start("ckv", ckv_h.at[0], ckv)
    for j in range(nch):
        start(f"wuk{j}", wuk_h.at[pl.ds(j * CCH, CCH)], wuk.at[pl.ds(j * CCH, CCH)])
        start(f"wuv{j}", wuv_h.at[pl.ds(j * CCH, CCH)], wuv.at[pl.ds(j * CCH, CCH)])
    start("wo", wo_h, wo)

    wait("ax", "fdr", "fdi")
    RC = 512
    for r in range(0, S, RC):
        a = ax[r:r + RC, :]
        x1r[r:r + RC, :] = _dot(a, fdr[...])
        x1i[r:r + RC, :] = _dot(a, fdi[...])

    lane_tiles = [(0, 128), (128, Df)]

    def radix16(src_r, src_i, dst_r, dst_i, sign):
        for b0 in range(0, RB, 8):
            for (l0, l1) in lane_tiles:
                xs = [(src_r[RB * a + b0:RB * a + b0 + 8, l0:l1],
                       src_i[RB * a + b0:RB * a + b0 + 8, l0:l1]) for a in range(NB)]
                ys = _dft16(xs, sign)
                for k in range(NB):
                    dst_r[RB * k + b0:RB * k + b0 + 8, l0:l1] = ys[k][0]
                    dst_i[RB * k + b0:RB * k + b0 + 8, l0:l1] = ys[k][1]

    radix16(x1r, x1i, x1r, x1i, -1)

    wait("wr", "wi", "gf", "gi")
    for src, dst in ((wr, wrp), (wi, wip)):
        for j in range(0, RB, 32):
            v = src[j * NB:(j + 32) * NB, :].reshape(32, NB, Df)
            dst[:, j:j + 32, :] = jnp.swapaxes(v, 0, 1)

    for k1 in range(NB):
        rows = slice(k1 * RB, (k1 + 1) * RB)
        g = gf[k1]
        pr = _dot(g, x1r[rows, :].astype(_BF16))
        pi = _dot(g, x1i[rows, :].astype(_BF16))
        xr = pr[:RB] - pi[RB:]
        xi = pr[RB:] + pi[:RB]
        w_r = wrp[k1].astype(_F32)
        w_i = wip[k1].astype(_F32)
        yr = (xr * w_r - xi * w_i).astype(_BF16)
        yi = (xr * w_i + xi * w_r).astype(_BF16)
        h = gi[k1]
        qr = _dot(h, yr)
        qi = _dot(h, yi)
        x1r[rows, :] = qr[:RB] + qi[RB:]
        x1i[rows, :] = qi[:RB] - qr[RB:]

    radix16(x1r, x1i, x1r, x1i, +1)

    wait("gdr", "gdi")
    for r in range(0, S, RC):
        ya = _dot(x1r[r:r + RC, :].astype(_BF16), gdr[...]) + _dot(x1i[r:r + RC, :].astype(_BF16), gdi[...])
        stage[r:r + RC, 0:M] = ya.astype(_BF16)

    wait("wq", "bx")
    for j in range(0, M, 64):
        wq_t[:, j:j + 64, :] = jnp.swapaxes(wq[j:j + 64], 0, 1)

    def deint(j):
        wait(f"wuk{j}", f"wuv{j}")
        rows = slice(j * CCH, (j + 1) * CCH)
        wkv_t[:, rows, 0:D] = jnp.swapaxes(wuk[rows], 0, 1)
        wkv_t[:, rows, D:2 * D] = jnp.swapaxes(wuv[rows], 0, 1)

    for h in range(H):
        for r in range(0, S, 1024):
            q_all[h, r:r + 1024, :] = _dot(bx[r:r + 1024, :], wq_t[h]).astype(_BF16)
        if h >= H - nch - 2 and h < H - 2:
            deint(h - (H - nch - 2))

    wait("ckv")
    for r in range(0, S, BQ):
        kv[0, r:r + BQ, :] = _dot(ckv[r:r + BQ, :], wkv_t[0]).astype(_BF16)
    wait("wo")
    acc[...] = jnp.zeros_like(acc)

    NQ = S // BQ
    SUB = 128
    nsub = BQ // SUB
    scale = _LOG2E * (D ** -0.5)

    def out_copy(i):
        return pltpu.make_async_copy(stage.at[pl.ds(i * BQ, BQ)], out_h.at[0, pl.ds(i * BQ, BQ)], osem.at[i])

    def head(h, last):
        slot = h % 2
        for i in range(NQ):
            r0, r1 = i * BQ, (i + 1) * BQ
            parts = []
            if i > 0:
                parts.append(_dot_nt(q_all[h, r0:r1, :], kv[slot, 0:r0, 0:D]))
            for t in range(nsub):
                c0 = r0 + t * SUB
                s = _dot_nt(q_all[h, c0:r1, :], kv[slot, c0:c0 + SUB, 0:D])
                ri = lax.broadcasted_iota(jnp.int32, (r1 - c0, SUB), 0)
                ci = lax.broadcasted_iota(jnp.int32, (r1 - c0, SUB), 1)
                s = jnp.where(ci <= ri, s, _NEG)
                if t > 0:
                    s = jnp.concatenate([jnp.full((c0 - r0, SUB), _NEG, _F32), s], 0)
                parts.append(s)
            s = jnp.concatenate(parts, 1)
            if not last:
                kv[1 - slot, r0:r1, :] = _dot(ckv[r0:r1, :], wkv_t[h + 1]).astype(_BF16)
            m = jnp.max(s, axis=1, keepdims=True)
            p = jnp.exp2((s - m) * scale)
            l = jnp.sum(p, axis=1, keepdims=True)
            pb = p.astype(_BF16)
            o = None
            if i > 0:
                o = _dot(pb[:, :r0], kv[slot, 0:r0, D:2 * D])
            for t in range(nsub):
                c0 = r0 + t * SUB
                ot = _dot(pb[t * SUB:, c0:c0 + SUB], kv[slot, c0:c0 + SUB, D:2 * D])
                if t > 0:
                    ot = jnp.concatenate([jnp.zeros((t * SUB, D), _F32), ot], 0)
                o = ot if o is None else o + ot
            o = o * (1.0 / l)
            res = acc[r0:r1, :] + _dot(o.astype(_BF16), wo[h])
            if last:
                stage[r0:r1, M:2 * M] = res.astype(_BF16)
                out_copy(i).start()
            else:
                acc[r0:r1, :] = res

    def body(h, c):
        head(h, False)
        return c

    lax.fori_loop(0, H - 1, body, 0)
    head(H - 1, True)
    for i in range(NQ):
        out_copy(i).wait()


@jax.jit
def pallas_concat_heads__spectral_gfnet__compressed_kv_cla__prompt_kernel(
    A_x: jax.Array,
    A_w_r: jax.Array,
    A_w_i: jax.Array,
    B_x: jax.Array,
    B_c_kv: jax.Array,
    B_w_q: jax.Array,
    B_w_uk: jax.Array,
    B_w_uv: jax.Array,
    B_w_o: jax.Array,
):
    B, S, M = A_x.shape
    Df = M // 2 + 1
    C = B_c_kv.shape[-1]
    _, H, D = B_w_q.shape
    BQ = 512
    tables = [jnp.asarray(t) for t in _dft_tables(S, M)]

    vm = pltpu.VMEM
    scratch = [
        vm((S, M), _BF16), vm((S, Df), _BF16), vm((S, Df), _BF16),
        vm((S, M), _BF16), vm((S, C), _BF16),
        vm((M, H, D), _BF16), vm((C, H, D), _BF16), vm((C, H, D), _BF16),
        vm((H, D, M), _BF16),
        vm((M, Df), _BF16), vm((M, Df), _BF16),
        vm((16, 256, 128), _BF16), vm((16, 256, 128), _BF16),
        vm((Df, M), _BF16), vm((Df, M), _BF16),
        vm((S, Df), _F32), vm((S, Df), _F32),
        vm((8, 128), _F32), vm((8, 128), _F32),
        vm((16, S // 16, Df), _BF16), vm((16, S // 16, Df), _BF16),
        vm((H, M, D), _BF16), vm((H, C, 2 * D), _BF16),
        vm((H, S, D), _BF16), vm((2, S, 2 * D), _BF16),
        vm((S, M), _F32), vm((S, 2 * M), _BF16),
        pltpu.SemaphoreType.DMA((32,)), pltpu.SemaphoreType.DMA((S // BQ,)),
    ]
    any_spec = pl.BlockSpec(memory_space=pltpu.HBM)
    return pl.pallas_call(
        functools.partial(_kernel, S=S, M=M, H=H, D=D, C=C, BQ=BQ),
        in_specs=[any_spec] * 15,
        out_specs=any_spec,
        out_shape=jax.ShapeDtypeStruct((B, S, 2 * M), _BF16),
        scratch_shapes=scratch,
        compiler_params=pltpu.CompilerParams(vmem_limit_bytes=120 * 2**20),
        name="gfnet_cla",
    )(A_x, A_w_r, A_w_i, B_x, B_c_kv, B_w_q, B_w_uk, B_w_uv, B_w_o, *tables)
```

```python
import functools

import jax
import jax.numpy as jnp
import numpy as np
from jax import lax
import jax.experimental.pallas as pl
import jax.experimental.pallas.tpu as pltpu

_BF16 = jnp.bfloat16
_F32 = jnp.float32
_NT = (((1,), (1,)), ((), ()))
_LOG2E = 1.4426950408889634
_NEG = -1e30


def _np_bf16(a):
    import ml_dtypes
    return np.asarray(a, np.float64).astype(np.float32).astype(ml_dtypes.bfloat16)


@functools.lru_cache(maxsize=None)
def _dft_tables(S, D):
    Df = D // 2 + 1
    n1, n2 = 16, S // 16
    d = np.arange(D)[:, None]
    c = np.arange(Df)[None, :]
    ang = 2.0 * np.pi * ((d * c) % D) / D
    fdr = np.cos(ang)
    fdi = -np.sin(ang)
    wgt = np.full(Df, 2.0)
    wgt[0] = 1.0
    if D % 2 == 0:
        wgt[-1] = 1.0
    gdr = wgt[:, None] * np.cos(ang.T) / (S * D)
    gdi = -wgt[:, None] * np.sin(ang.T) / (S * D)
    k1 = np.arange(n1)[:, None, None]
    k2 = np.arange(n2)[None, :, None]
    b = np.arange(n2)[None, None, :]
    g = np.exp(-2j * np.pi * ((b * (k1 + n1 * k2)) % S) / S)
    gf = np.concatenate([g.real, g.imag], axis=1)
    gt = np.transpose(g, (0, 2, 1))
    gi = np.concatenate([gt.real, gt.imag], axis=1)
    hr = -(-Df // 8) * 8
    fdt = np.zeros((2 * hr, D))
    fdt[:Df] = fdr.T
    fdt[hr:hr + Df] = fdi.T
    return tuple(_np_bf16(t) for t in (fdt, gf, gi, gdr, gdi))


_R2 = float(np.sqrt(0.5))
_C1, _S1 = float(np.cos(np.pi / 8)), float(np.sin(np.pi / 8))


def _cmul(ar, ai, wr, wi):
    return ar * wr - ai * wi, ar * wi + ai * wr


def _tw16(ar, ai, e, sign):
    e %= 16
    if e == 0:
        return ar, ai
    if e == 4:
        return (-ai, ar) if sign > 0 else (ai, -ar)
    if e == 2:
        return ((ar - ai) * _R2, (ar + ai) * _R2) if sign > 0 else ((ar + ai) * _R2, (ai - ar) * _R2)
    if e == 6:
        return ((-ar - ai) * _R2, (ar - ai) * _R2) if sign > 0 else ((ai - ar) * _R2, (-ar - ai) * _R2)
    ang = sign * 2.0 * np.pi * e / 16
    return _cmul(ar, ai, float(np.cos(ang)), float(np.sin(ang)))


def _dft4(x, sign):
    (ar, ai), (br, bi), (cr, ci), (dr, di) = x
    t0r, t0i = ar + cr, ai + ci
    t1r, t1i = ar - cr, ai - ci
    t2r, t2i = br + dr, bi + di
    t3r, t3i = br - dr, bi - di
    y0 = (t0r + t2r, t0i + t2i)
    y2 = (t0r - t2r, t0i - t2i)
    if sign < 0:
        y1 = (t1r + t3i, t1i - t3r)
        y3 = (t1r - t3i, t1i + t3r)
    else:
        y1 = (t1r - t3i, t1i + t3r)
        y3 = (t1r + t3i, t1i - t3r)
    return [y0, y1, y2, y3]


def _dft16(x, sign):
    cols = []
    for n2 in range(4):
        y = _dft4([x[4 * n1 + n2] for n1 in range(4)], sign)
        cols.append([_tw16(y[k1][0], y[k1][1], n2 * k1, sign) for k1 in range(4)])
    out = [None] * 16
    for k1 in range(4):
        z = _dft4([cols[n2][k1] for n2 in range(4)], sign)
        for k2 in range(4):
            out[k1 + 4 * k2] = z[k2]
    return out


def _dot(a, b):
    return jnp.dot(a, b, preferred_element_type=_F32)


def _dot_nt(a, b):
    return lax.dot_general(a, b, _NT, preferred_element_type=_F32)


def _kernel(ax_h, wr_h, wi_h, bx_h, ckv_h, wq_h, wuk_h, wuv_h, wo_h,
            fdt_h, gf_h, gi_h, gdr_h, gdi_h,
            out_h,
            axt, wrt, wit, bxt, ckv, wq, wuk, wuv, wot, fdt, gf, gi, gdr, gdi,
            x1t, zr, zi, wrp, wip, bx,
            wq_t, wkv_t, q_all, kv, acc, stage, sem, osem,
            *, S, M, H, D, C, BQ):
    Df = M // 2 + 1
    NB = 16
    RB = S // NB
    CCH = 128
    nch = C // CCH

    copies = {}
    sem_ids = {}

    def start(name, src, dst):
        i = len(sem_ids)
        sem_ids[name] = i
        cp = pltpu.make_async_copy(src, dst, sem.at[i])
        cp.start()
        copies[name] = cp

    def wait(*names):
        for n in names:
            copies[n].wait()

    start("ax", ax_h.at[0], axt)
    start("fdt", fdt_h, fdt)
    start("gf", gf_h, gf)
    start("wr", wr_h, wrt)
    start("wi", wi_h, wit)
    start("gi", gi_h, gi)
    start("gdr", gdr_h, gdr)
    start("gdi", gdi_h, gdi)
    start("wq", wq_h, wq)
    start("bx", bx_h.at[0], bxt)
    start("ckv", ckv_h.at[0], ckv)
    for j in range(nch):
        start(f"wuk{j}", wuk_h.at[pl.ds(j * CCH, CCH)], wuk.at[pl.ds(j * CCH, CCH)])
        start(f"wuv{j}", wuv_h.at[pl.ds(j * CCH, CCH)], wuv.at[pl.ds(j * CCH, CCH)])
    start("wo", wo_h, wot)

    wait("ax", "fdt")
    RC = 512
    HR = -(-Df // 8) * 8
    for c0 in range(0, S, RC):
        x1t[:, c0:c0 + RC] = _dot(fdt[...], axt[:, c0:c0 + RC])

    for g in range(0, HR, 8):
        xs = [(x1t[g:g + 8, RB * a:RB * (a + 1)], x1t[HR + g:HR + g + 8, RB * a:RB * (a + 1)])
              for a in range(NB)]
        ys = _dft16(xs, -1)
        for k in range(NB):
            x1t[g:g + 8, RB * k:RB * (k + 1)] = ys[k][0]
            x1t[HR + g:HR + g + 8, RB * k:RB * (k + 1)] = ys[k][1]

    wait("wr", "wi", "gf", "gi")
    for src, dst in ((wrt, wrp), (wit, wip)):
        for j in range(0, RB, 32):
            v = src[:, j * NB:(j + 32) * NB].T.reshape(32, NB, Df)
            dst[:, j:j + 32, :] = jnp.swapaxes(v, 0, 1)

    for k1 in range(NB):
        rows = slice(k1 * RB, (k1 + 1) * RB)
        g = gf[k1]
        pr = _dot_nt(g, x1t[0:Df, rows].astype(_BF16))
        pi = _dot_nt(g, x1t[HR:HR + Df, rows].astype(_BF16))
        xr = pr[:RB] - pi[RB:]
        xi = pr[RB:] + pi[:RB]
        w_r = wrp[k1].astype(_F32)
        w_i = wip[k1].astype(_F32)
        yr = (xr * w_r - xi * w_i).astype(_BF16)
        yi = (xr * w_i + xi * w_r).astype(_BF16)
        h = gi[k1]
        qr = _dot(h, yr)
        qi = _dot(h, yi)
        zr[rows, :] = qr[:RB] + qi[RB:]
        zi[rows, :] = qi[:RB] - qr[RB:]

    for b0 in range(0, RB, 8):
        for (l0, l1) in ((0, 128), (128, Df)):
            xs = [(zr[RB * a + b0:RB * a + b0 + 8, l0:l1], zi[RB * a + b0:RB * a + b0 + 8, l0:l1])
                  for a in range(NB)]
            ys = _dft16(xs, +1)
            for k in range(NB):
                zr[RB * k + b0:RB * k + b0 + 8, l0:l1] = ys[k][0]
                zi[RB * k + b0:RB * k + b0 + 8, l0:l1] = ys[k][1]

    wait("gdr", "gdi")
    for r in range(0, S, RC):
        ya = _dot(zr[r:r + RC, :].astype(_BF16), gdr[...]) + _dot(zi[r:r + RC, :].astype(_BF16), gdi[...])
        stage[r:r + RC, 0:M] = ya.astype(_BF16)

    wait("wq", "bx")
    for c0 in range(0, S, RC):
        bx[c0:c0 + RC, :] = bxt[:, c0:c0 + RC].T
    for j in range(0, M, 64):
        wq_t[:, j:j + 64, :] = jnp.swapaxes(wq[j:j + 64], 0, 1)

    def deint(j):
        wait(f"wuk{j}", f"wuv{j}")
        rows = slice(j * CCH, (j + 1) * CCH)
        wkv_t[:, rows, 0:D] = jnp.swapaxes(wuk[rows], 0, 1)
        wkv_t[:, rows, D:2 * D] = jnp.swapaxes(wuv[rows], 0, 1)

    for h in range(H):
        for r in range(0, S, 1024):
            q_all[h, r:r + 1024, :] = _dot(bx[r:r + 1024, :], wq_t[h]).astype(_BF16)
        if h >= H - nch - 2 and h < H - 2:
            deint(h - (H - nch - 2))

    wait("ckv")
    for r in range(0, S, BQ):
        kv[0, r:r + BQ, :] = _dot(ckv[r:r + BQ, :], wkv_t[0]).astype(_BF16)
    wait("wo")
    acc[...] = jnp.zeros_like(acc)

    NQ = S // BQ
    SUB = 128
    nsub = BQ // SUB
    scale = _LOG2E * (D ** -0.5)

    def out_copy(i):
        return pltpu.make_async_copy(stage.at[pl.ds(i * BQ, BQ)], out_h.at[0, pl.ds(i * BQ, BQ)], osem.at[i])

    def head(h, last):
        slot = h % 2
        for i in range(NQ):
            r0, r1 = i * BQ, (i + 1) * BQ
            parts = []
            if i > 0:
                parts.append(_dot_nt(q_all[h, r0:r1, :], kv[slot, 0:r0, 0:D]))
            for t in range(nsub):
                c0 = r0 + t * SUB
                s = _dot_nt(q_all[h, c0:r1, :], kv[slot, c0:c0 + SUB, 0:D])
                ri = lax.broadcasted_iota(jnp.int32, (r1 - c0, SUB), 0)
                ci = lax.broadcasted_iota(jnp.int32, (r1 - c0, SUB), 1)
                s = jnp.where(ci <= ri, s, _NEG)
                if t > 0:
                    s = jnp.concatenate([jnp.full((c0 - r0, SUB), _NEG, _F32), s], 0)
                parts.append(s)
            s = jnp.concatenate(parts, 1)
            if not last:
                kv[1 - slot, r0:r1, :] = _dot(ckv[r0:r1, :], wkv_t[h + 1]).astype(_BF16)
            m = jnp.max(s, axis=1, keepdims=True)
            p = jnp.exp2((s - m) * scale)
            l = jnp.sum(p, axis=1, keepdims=True)
            pb = p.astype(_BF16)
            o = None
            if i > 0:
                o = _dot(pb[:, :r0], kv[slot, 0:r0, D:2 * D])
            for t in range(nsub):
                c0 = r0 + t * SUB
                ot = _dot(pb[t * SUB:, c0:c0 + SUB], kv[slot, c0:c0 + SUB, D:2 * D])
                if t > 0:
                    ot = jnp.concatenate([jnp.zeros((t * SUB, D), _F32), ot], 0)
                o = ot if o is None else o + ot
            o = o * (1.0 / l)
            res = acc[:, r0:r1] + _dot_nt(wot[h], o.astype(_BF16))
            if last:
                stage[r0:r1, M:2 * M] = res.astype(_BF16).T
                out_copy(i).start()
            else:
                acc[:, r0:r1] = res

    def body(h, c):
        head(h, False)
        return c

    lax.fori_loop(0, H - 1, body, 0)
    head(H - 1, True)
    for i in range(NQ):
        out_copy(i).wait()


@jax.jit
def pallas_concat_heads__spectral_gfnet__compressed_kv_cla__prompt_kernel(
    A_x: jax.Array,
    A_w_r: jax.Array,
    A_w_i: jax.Array,
    B_x: jax.Array,
    B_c_kv: jax.Array,
    B_w_q: jax.Array,
    B_w_uk: jax.Array,
    B_w_uv: jax.Array,
    B_w_o: jax.Array,
):
    B, S, M = A_x.shape
    Df = M // 2 + 1
    C = B_c_kv.shape[-1]
    _, H, D = B_w_q.shape
    BQ = 512
    tables = [jnp.asarray(t) for t in _dft_tables(S, M)]

    vm = pltpu.VMEM
    HR = -(-Df // 8) * 8
    scratch = [
        vm((M, S), _BF16), vm((Df, S), _BF16), vm((Df, S), _BF16),
        vm((M, S), _BF16), vm((S, C), _BF16),
        vm((M, H, D), _BF16), vm((C, H, D), _BF16), vm((C, H, D), _BF16),
        vm((H, M, D), _BF16),
        vm((2 * HR, M), _BF16),
        vm((16, 256, 128), _BF16), vm((16, 256, 128), _BF16),
        vm((Df, M), _BF16), vm((Df, M), _BF16),
        vm((2 * HR, S), _F32), vm((S, Df), _F32), vm((S, Df), _F32),
        vm((16, S // 16, Df), _BF16), vm((16, S // 16, Df), _BF16),
        vm((S, M), _BF16),
        vm((H, M, D), _BF16), vm((H, C, 2 * D), _BF16),
        vm((H, S, D), _BF16), vm((2, S, 2 * D), _BF16),
        vm((M, S), _F32), vm((S, 2 * M), _BF16),
        pltpu.SemaphoreType.DMA((32,)), pltpu.SemaphoreType.DMA((S // BQ,)),
    ]
    any_spec = pl.BlockSpec(memory_space=pltpu.HBM)
    return pl.pallas_call(
        functools.partial(_kernel, S=S, M=M, H=H, D=D, C=C, BQ=BQ),
        in_specs=[any_spec] * 14,
        out_specs=any_spec,
        out_shape=jax.ShapeDtypeStruct((B, S, 2 * M), _BF16),
        scratch_shapes=scratch,
        compiler_params=pltpu.CompilerParams(vmem_limit_bytes=120 * 2**20),
        name="gfnet_cla",
    )(jnp.swapaxes(A_x, 1, 2), A_w_r.T, A_w_i.T, jnp.swapaxes(B_x, 1, 2), B_c_kv,
      B_w_q, B_w_uk, B_w_uv, jnp.swapaxes(B_w_o, 1, 2), *tables)
```

```python
import functools

import jax
import jax.numpy as jnp
import numpy as np
from jax import lax
import jax.experimental.pallas as pl
import jax.experimental.pallas.tpu as pltpu

_BF16 = jnp.bfloat16
_F32 = jnp.float32
_NT = (((1,), (1,)), ((), ()))
_LOG2E = 1.4426950408889634
_NEG = -1e30


def _np_bf16(a):
    import ml_dtypes
    return np.asarray(a, np.float64).astype(np.float32).astype(ml_dtypes.bfloat16)


@functools.lru_cache(maxsize=None)
def _dft_tables(S, D):
    Df = D // 2 + 1
    n1, n2 = 16, S // 16
    d = np.arange(D)[:, None]
    c = np.arange(Df)[None, :]
    ang = 2.0 * np.pi * ((d * c) % D) / D
    fdr = np.cos(ang)
    fdi = -np.sin(ang)
    wgt = np.full(Df, 2.0)
    wgt[0] = 1.0
    if D % 2 == 0:
        wgt[-1] = 1.0
    gdr = wgt[:, None] * np.cos(ang.T) / (S * D)
    gdi = -wgt[:, None] * np.sin(ang.T) / (S * D)
    k1 = np.arange(n1)[:, None, None]
    k2 = np.arange(n2)[None, :, None]
    b = np.arange(n2)[None, None, :]
    g = np.exp(-2j * np.pi * ((b * (k1 + n1 * k2)) % S) / S)
    gf = np.concatenate([g.real, g.imag], axis=1)
    gt = np.transpose(g, (0, 2, 1))
    gi = np.concatenate([gt.real, gt.imag], axis=1)
    hr = -(-Df // 8) * 8
    fdt = np.zeros((2 * hr, D))
    fdt[:Df] = fdr.T
    fdt[hr:hr + Df] = fdi.T
    return tuple(_np_bf16(t) for t in (fdt, gf, gi, gdr, gdi))


_R2 = float(np.sqrt(0.5))
_C1, _S1 = float(np.cos(np.pi / 8)), float(np.sin(np.pi / 8))


def _cmul(ar, ai, wr, wi):
    return ar * wr - ai * wi, ar * wi + ai * wr


def _tw16(ar, ai, e, sign):
    e %= 16
    if e == 0:
        return ar, ai
    if e == 4:
        return (-ai, ar) if sign > 0 else (ai, -ar)
    if e == 2:
        return ((ar - ai) * _R2, (ar + ai) * _R2) if sign > 0 else ((ar + ai) * _R2, (ai - ar) * _R2)
    if e == 6:
        return ((-ar - ai) * _R2, (ar - ai) * _R2) if sign > 0 else ((ai - ar) * _R2, (-ar - ai) * _R2)
    ang = sign * 2.0 * np.pi * e / 16
    return _cmul(ar, ai, float(np.cos(ang)), float(np.sin(ang)))


def _dft4(x, sign):
    (ar, ai), (br, bi), (cr, ci), (dr, di) = x
    t0r, t0i = ar + cr, ai + ci
    t1r, t1i = ar - cr, ai - ci
    t2r, t2i = br + dr, bi + di
    t3r, t3i = br - dr, bi - di
    y0 = (t0r + t2r, t0i + t2i)
    y2 = (t0r - t2r, t0i - t2i)
    if sign < 0:
        y1 = (t1r + t3i, t1i - t3r)
        y3 = (t1r - t3i, t1i + t3r)
    else:
        y1 = (t1r - t3i, t1i + t3r)
        y3 = (t1r + t3i, t1i - t3r)
    return [y0, y1, y2, y3]


def _dft16(x, sign):
    cols = []
    for n2 in range(4):
        y = _dft4([x[4 * n1 + n2] for n1 in range(4)], sign)
        cols.append([_tw16(y[k1][0], y[k1][1], n2 * k1, sign) for k1 in range(4)])
    out = [None] * 16
    for k1 in range(4):
        z = _dft4([cols[n2][k1] for n2 in range(4)], sign)
        for k2 in range(4):
            out[k1 + 4 * k2] = z[k2]
    return out


def _dot(a, b):
    return jnp.dot(a, b, preferred_element_type=_F32)


def _dot_nt(a, b):
    return lax.dot_general(a, b, _NT, preferred_element_type=_F32)


def _weave(main, side):
    k = 0
    for j, f in enumerate(main):
        f()
        upto = len(side) * (j + 1) // len(main)
        while k < upto:
            side[k]()
            k += 1
    for f in side[k:]:
        f()


def _kernel(ax_h, wr_h, wi_h, bx_h, ckv_h, wq_h, wuk_h, wuv_h, wo_h,
            fdt_h, gf_h, gi_h, gdr_h, gdi_h,
            out_h,
            axt, wrt, wit, bxt, ckv, wq, wuk, wuv, wot, fdt, gf, gi, gdr, gdi,
            x1t, zr, zi, wrp, wip, bx,
            wq_t, wkv_t, q_all, kv, acc, stage, sbuf, pbuf, cbuf, sem, osem,
            *, S, M, H, D, C, BQ):
    Df = M // 2 + 1
    NB = 16
    RB = S // NB
    CCH = 128
    nch = C // CCH

    copies = {}
    sem_ids = {}

    def start(name, src, dst):
        i = len(sem_ids)
        sem_ids[name] = i
        cp = pltpu.make_async_copy(src, dst, sem.at[i])
        cp.start()
        copies[name] = cp

    def wait(*names):
        for n in names:
            copies[n].wait()

    start("ax", ax_h.at[0], axt)
    start("fdt", fdt_h, fdt)
    start("gf", gf_h, gf)
    start("wr", wr_h, wrt)
    start("wi", wi_h, wit)
    start("gi", gi_h, gi)
    start("gdr", gdr_h, gdr)
    start("gdi", gdi_h, gdi)
    start("wq", wq_h, wq)
    start("bx", bx_h.at[0], bxt)

    def chunk_copies(j):
        rows = pl.ds(j * CCH, CCH)
        return (pltpu.make_async_copy(wuk_h.at[rows], wuk.at[rows], sem.at[16 + 2 * j]),
                pltpu.make_async_copy(wuv_h.at[rows], wuv.at[rows], sem.at[17 + 2 * j]))

    for j in range(nch):
        for cp in chunk_copies(j):
            cp.start()
    start("ckv", ckv_h.at[0], ckv)
    start("wo", wo_h, wot)

    wait("ax", "fdt")
    RC = 512
    HR = -(-Df // 8) * 8
    for c0 in range(0, S, RC):
        x1t[:, c0:c0 + RC] = _dot(fdt[...], axt[:, c0:c0 + RC])

    for g in range(0, HR, 8):
        xs = [(x1t[g:g + 8, RB * a:RB * (a + 1)], x1t[HR + g:HR + g + 8, RB * a:RB * (a + 1)])
              for a in range(NB)]
        ys = _dft16(xs, -1)
        for k in range(NB):
            x1t[g:g + 8, RB * k:RB * (k + 1)] = ys[k][0]
            x1t[HR + g:HR + g + 8, RB * k:RB * (k + 1)] = ys[k][1]

    wait("wr", "wi", "gf", "gi")
    for src, dst in ((wrt, wrp), (wit, wip)):
        for j in range(0, RB, 32):
            v = src[:, j * NB:(j + 32) * NB].T.reshape(32, NB, Df)
            dst[:, j:j + 32, :] = jnp.swapaxes(v, 0, 1)

    for k1 in range(NB):
        rows = slice(k1 * RB, (k1 + 1) * RB)
        g = gf[k1]
        pr = _dot_nt(g, x1t[0:Df, rows].astype(_BF16))
        pi = _dot_nt(g, x1t[HR:HR + Df, rows].astype(_BF16))
        xr = pr[:RB] - pi[RB:]
        xi = pr[RB:] + pi[:RB]
        w_r = wrp[k1].astype(_F32)
        w_i = wip[k1].astype(_F32)
        yr = (xr * w_r - xi * w_i).astype(_BF16)
        yi = (xr * w_i + xi * w_r).astype(_BF16)
        h = gi[k1]
        qr = _dot(h, yr)
        qi = _dot(h, yi)
        zr[rows, :] = qr[:RB] + qi[RB:]
        zi[rows, :] = qi[:RB] - qr[RB:]

    for b0 in range(0, RB, 8):
        for (l0, l1) in ((0, 128), (128, Df)):
            xs = [(zr[RB * a + b0:RB * a + b0 + 8, l0:l1], zi[RB * a + b0:RB * a + b0 + 8, l0:l1])
                  for a in range(NB)]
            ys = _dft16(xs, +1)
            for k in range(NB):
                zr[RB * k + b0:RB * k + b0 + 8, l0:l1] = ys[k][0]
                zi[RB * k + b0:RB * k + b0 + 8, l0:l1] = ys[k][1]

    wait("gdr", "gdi")
    for r in range(0, S, RC):
        ya = _dot(zr[r:r + RC, :].astype(_BF16), gdr[...]) + _dot(zi[r:r + RC, :].astype(_BF16), gdi[...])
        stage[r:r + RC, 0:M] = ya.astype(_BF16)

    wait("wq", "bx")
    for c0 in range(0, S, RC):
        bx[c0:c0 + RC, :] = bxt[:, c0:c0 + RC].T
    for j in range(0, M, 64):
        wq_t[:, j:j + 64, :] = jnp.swapaxes(wq[j:j + 64], 0, 1)

    QR = 256
    DR = 16

    def qbody(j, c):
        jj = pl.multiple_of(j * CCH, CCH)

        def qtask(hh, r):
            def f():
                q_all[hh, r:r + QR, :] = _dot(bx[r:r + QR, :], wq_t[hh]).astype(_BF16)
            return f

        def dtask(src, lane0, u):
            def f():
                rows = pl.ds(pl.multiple_of(jj + u, DR), DR)
                wkv_t[:, rows, lane0:lane0 + D] = jnp.swapaxes(src[rows], 0, 1)
            return f

        for r in range(0, S, QR):
            qtask(2 * j, r)()
        for cp in chunk_copies(j):
            cp.wait()
        side = [dtask(src, l0, u) for u in range(0, CCH, DR) for (src, l0) in ((wuk, 0), (wuv, D))]
        _weave([qtask(2 * j + 1, r) for r in range(0, S, QR)], side)
        return c

    for j in range(nch):
        qbody(j, 0)

    wait("ckv")

    def kv0body(j, c):
        rows = pl.ds(pl.multiple_of(j * BQ, BQ), BQ)
        kv[0, rows, :] = _dot(ckv[rows, :], wkv_t[0]).astype(_BF16)
        return c

    for j in range(S // BQ):
        kv0body(j, 0)
    wait("wo")
    acc[...] = jnp.zeros_like(acc)

    NQ = S // BQ
    SUB = 128
    nsub = BQ // SUB
    scale = _LOG2E * (D ** -0.5)

    def out_copy(i):
        return pltpu.make_async_copy(stage.at[pl.ds(i * BQ, BQ)], out_h.at[0, pl.ds(i * BQ, BQ)], osem.at[i])

    RH = 128
    order = list(range(NQ))[::-1]

    def head(h, last):
        slot = h % 2
        ls = {}

        def s_tasks(i, par):
            r0, r1 = i * BQ, (i + 1) * BQ
            ts = []
            for c0 in range(0, r0, BQ):
                def f(c0=c0):
                    sbuf[par, :, c0:c0 + BQ] = _dot_nt(q_all[h, r0:r1, :], kv[slot, c0:c0 + BQ, 0:D])
                ts.append(f)
            for t in range(nsub):
                def f(t=t):
                    c0 = r0 + t * SUB
                    sc = _dot_nt(q_all[h, c0:r1, :], kv[slot, c0:c0 + SUB, 0:D])
                    ri = lax.broadcasted_iota(jnp.int32, (SUB, SUB), 0)
                    ci = lax.broadcasted_iota(jnp.int32, (SUB, SUB), 1)
                    sbuf[par, t * SUB:(t + 1) * SUB, c0:c0 + SUB] = jnp.where(ci <= ri, sc[:SUB], _NEG)
                    if t + 1 < nsub:
                        sbuf[par, (t + 1) * SUB:, c0:c0 + SUB] = sc[SUB:]
                ts.append(f)
            return ts

        def sm_tasks(i, par):
            ts = []
            for j in range(BQ // RH):
                def f(j=j):
                    kvl = i * BQ + (j + 1) * RH
                    sc = sbuf[par, j * RH:(j + 1) * RH, 0:kvl]
                    m = jnp.max(sc, axis=1, keepdims=True)
                    p = jnp.exp2((sc - m) * scale)
                    ls[(i, j)] = jnp.sum(p, axis=1, keepdims=True)
                    pbuf[par, j * RH:(j + 1) * RH, 0:kvl] = p.astype(_BF16)
                ts.append(f)
            return ts

        def pv_tasks(i, par):
            ts = []
            for j in range(BQ // RH):
                def f(j=j):
                    kvl = i * BQ + (j + 1) * RH
                    o = _dot(pbuf[par, j * RH:(j + 1) * RH, 0:kvl], kv[slot, 0:kvl, D:2 * D])
                    cbuf[par, j * RH:(j + 1) * RH, :] = (o * (1.0 / ls[(i, j)])).astype(_BF16)
                ts.append(f)
            return ts

        def op_tasks(i, par):
            def f():
                r0, r1 = i * BQ, (i + 1) * BQ
                res = acc[:, r0:r1] + _dot_nt(wot[h], cbuf[par])
                if last:
                    stage[r0:r1, M:2 * M] = res.astype(_BF16).T
                    out_copy(i).start()
                else:
                    acc[:, r0:r1] = res
            return [f]

        def kv_tasks(i):
            ts = []
            for u in range(0, BQ, 256):
                def f(u=u):
                    rows = slice(i * BQ + u, i * BQ + u + 256)
                    kv[1 - slot, rows, :] = _dot(ckv[rows, :], wkv_t[h + 1]).astype(_BF16)
                ts.append(f)
            return ts

        for f in s_tasks(order[0], 0):
            f()
        for n in range(NQ + 2):
            mx = s_tasks(order[n + 1], (n + 1) % 2) if n + 1 < NQ else []
            mx2 = []
            if 0 <= n - 2 < NQ:
                mx2 += op_tasks(order[n - 2], n % 2)
            if 0 <= n - 1 < NQ:
                mx2 += pv_tasks(order[n - 1], (n - 1) % 2)
            if n < NQ and not last:
                mx2 += kv_tasks(order[n])
            allm = []
            a = b = 0
            while a < len(mx) or b < len(mx2):
                if b >= len(mx2) or (a < len(mx) and a * len(mx2) <= b * len(mx)):
                    allm.append(mx[a])
                    a += 1
                else:
                    allm.append(mx2[b])
                    b += 1
            if n < NQ:
                _weave(sm_tasks(order[n], n % 2), allm)
            else:
                for f in allm:
                    f()

    def body(h, c):
        head(h, False)
        return c

    lax.fori_loop(0, H - 1, body, 0)
    head(H - 1, True)
    for i in range(NQ):
        out_copy(i).wait()


@jax.jit
def pallas_concat_heads__spectral_gfnet__compressed_kv_cla__prompt_kernel(
    A_x: jax.Array,
    A_w_r: jax.Array,
    A_w_i: jax.Array,
    B_x: jax.Array,
    B_c_kv: jax.Array,
    B_w_q: jax.Array,
    B_w_uk: jax.Array,
    B_w_uv: jax.Array,
    B_w_o: jax.Array,
):
    B, S, M = A_x.shape
    Df = M // 2 + 1
    C = B_c_kv.shape[-1]
    _, H, D = B_w_q.shape
    BQ = 512
    tables = [jnp.asarray(t) for t in _dft_tables(S, M)]

    vm = pltpu.VMEM
    HR = -(-Df // 8) * 8
    scratch = [
        vm((M, S), _BF16), vm((Df, S), _BF16), vm((Df, S), _BF16),
        vm((M, S), _BF16), vm((S, C), _BF16),
        vm((M, H, D), _BF16), vm((C, H, D), _BF16), vm((C, H, D), _BF16),
        vm((H, M, D), _BF16),
        vm((2 * HR, M), _BF16),
        vm((16, 256, 128), _BF16), vm((16, 256, 128), _BF16),
        vm((Df, M), _BF16), vm((Df, M), _BF16),
        vm((2 * HR, S), _F32), vm((S, Df), _F32), vm((S, Df), _F32),
        vm((16, S // 16, Df), _BF16), vm((16, S // 16, Df), _BF16),
        vm((S, M), _BF16),
        vm((H, M, D), _BF16), vm((H, C, 2 * D), _BF16),
        vm((H, S, D), _BF16), vm((2, S, 2 * D), _BF16),
        vm((M, S), _F32), vm((S, 2 * M), _BF16),
        vm((2, BQ, S), _F32), vm((2, BQ, S), _BF16), vm((2, BQ, D), _BF16),
        pltpu.SemaphoreType.DMA((16 + 2 * (C // 128),)),
        pltpu.SemaphoreType.DMA((S // BQ,)),
    ]
    any_spec = pl.BlockSpec(memory_space=pltpu.HBM)
    return pl.pallas_call(
        functools.partial(_kernel, S=S, M=M, H=H, D=D, C=C, BQ=BQ),
        in_specs=[any_spec] * 14,
        out_specs=any_spec,
        out_shape=jax.ShapeDtypeStruct((B, S, 2 * M), _BF16),
        scratch_shapes=scratch,
        compiler_params=pltpu.CompilerParams(vmem_limit_bytes=120 * 2**20),
        name="gfnet_cla",
    )(jnp.swapaxes(A_x, 1, 2), A_w_r.T, A_w_i.T, jnp.swapaxes(B_x, 1, 2), B_c_kv,
      B_w_q, B_w_uk, B_w_uv, jnp.swapaxes(B_w_o, 1, 2), *tables)
```

```python
import functools

import jax
import jax.numpy as jnp
import numpy as np
from jax import lax
import jax.experimental.pallas as pl
import jax.experimental.pallas.tpu as pltpu

_BF16 = jnp.bfloat16
_F32 = jnp.float32
_NT = (((1,), (1,)), ((), ()))
_LOG2E = 1.4426950408889634
_NEG = -1e30


def _np_bf16(a):
    import ml_dtypes
    return np.asarray(a, np.float64).astype(np.float32).astype(ml_dtypes.bfloat16)


@functools.lru_cache(maxsize=None)
def _dft_tables(S, D):
    Df = D // 2 + 1
    n1, n2 = 16, S // 16
    d = np.arange(D)[:, None]
    c = np.arange(Df)[None, :]
    ang = 2.0 * np.pi * ((d * c) % D) / D
    fdr = np.cos(ang)
    fdi = -np.sin(ang)
    wgt = np.full(Df, 2.0)
    wgt[0] = 1.0
    if D % 2 == 0:
        wgt[-1] = 1.0
    gdr = wgt[:, None] * np.cos(ang.T) / (S * D)
    gdi = -wgt[:, None] * np.sin(ang.T) / (S * D)
    k1 = np.arange(n1)[:, None, None]
    k2 = np.arange(n2)[None, :, None]
    b = np.arange(n2)[None, None, :]
    g = np.exp(-2j * np.pi * ((b * (k1 + n1 * k2)) % S) / S)
    gf = np.concatenate([g.real, g.imag], axis=1)
    gt = np.transpose(g, (0, 2, 1))
    gi = np.concatenate([gt.real, gt.imag], axis=1)
    hr = -(-Df // 8) * 8
    fdt = np.zeros((2 * hr, D))
    fdt[:Df] = fdr.T
    fdt[hr:hr + Df] = fdi.T
    return tuple(_np_bf16(t) for t in (fdt, gf, gi, gdr, gdi))


_R2 = float(np.sqrt(0.5))
_C1, _S1 = float(np.cos(np.pi / 8)), float(np.sin(np.pi / 8))


def _cmul(ar, ai, wr, wi):
    return ar * wr - ai * wi, ar * wi + ai * wr


def _tw16(ar, ai, e, sign):
    e %= 16
    if e == 0:
        return ar, ai
    if e == 4:
        return (-ai, ar) if sign > 0 else (ai, -ar)
    if e == 2:
        return ((ar - ai) * _R2, (ar + ai) * _R2) if sign > 0 else ((ar + ai) * _R2, (ai - ar) * _R2)
    if e == 6:
        return ((-ar - ai) * _R2, (ar - ai) * _R2) if sign > 0 else ((ai - ar) * _R2, (-ar - ai) * _R2)
    ang = sign * 2.0 * np.pi * e / 16
    return _cmul(ar, ai, float(np.cos(ang)), float(np.sin(ang)))


def _dft4(x, sign):
    (ar, ai), (br, bi), (cr, ci), (dr, di) = x
    t0r, t0i = ar + cr, ai + ci
    t1r, t1i = ar - cr, ai - ci
    t2r, t2i = br + dr, bi + di
    t3r, t3i = br - dr, bi - di
    y0 = (t0r + t2r, t0i + t2i)
    y2 = (t0r - t2r, t0i - t2i)
    if sign < 0:
        y1 = (t1r + t3i, t1i - t3r)
        y3 = (t1r - t3i, t1i + t3r)
    else:
        y1 = (t1r - t3i, t1i + t3r)
        y3 = (t1r + t3i, t1i - t3r)
    return [y0, y1, y2, y3]


def _dft16(x, sign):
    cols = []
    for n2 in range(4):
        y = _dft4([x[4 * n1 + n2] for n1 in range(4)], sign)
        cols.append([_tw16(y[k1][0], y[k1][1], n2 * k1, sign) for k1 in range(4)])
    out = [None] * 16
    for k1 in range(4):
        z = _dft4([cols[n2][k1] for n2 in range(4)], sign)
        for k2 in range(4):
            out[k1 + 4 * k2] = z[k2]
    return out


def _dot(a, b):
    return jnp.dot(a, b, preferred_element_type=_F32)


def _dot_nt(a, b):
    return lax.dot_general(a, b, _NT, preferred_element_type=_F32)


def _weave(main, side):
    k = 0
    for j, f in enumerate(main):
        f()
        upto = len(side) * (j + 1) // len(main)
        while k < upto:
            side[k]()
            k += 1
    for f in side[k:]:
        f()


def _kernel(ax_h, wr_h, wi_h, bx_h, ckv_h, wq_h, wuk_h, wuv_h, wo_h,
            fdt_h, gf_h, gi_h, gdr_h, gdi_h,
            out_h,
            axt, wrt, wit, bxt, ckv, wq, wuk, wuv, wot, fdt, gf, gi, gdr, gdi,
            x1t, zr, zi, wrp, wip, bx,
            wq_t, wkv_t, q_all, kv, acc, stage, sbuf, pbuf, cbuf, ac, sem, osem,
            *, S, M, H, D, C, BQ):
    Df = M // 2 + 1
    NB = 16
    RB = S // NB
    CCH = 128
    nch = C // CCH

    copies = {}
    sem_ids = {}

    def start(name, src, dst):
        i = len(sem_ids)
        sem_ids[name] = i
        cp = pltpu.make_async_copy(src, dst, sem.at[i])
        cp.start()
        copies[name] = cp

    def wait(*names):
        for n in names:
            copies[n].wait()

    start("ax", ax_h.at[0], axt)
    start("fdt", fdt_h, fdt)
    start("gf", gf_h, gf)
    start("wr", wr_h, wrt)
    start("wi", wi_h, wit)
    start("gi", gi_h, gi)
    start("gdr", gdr_h, gdr)
    start("gdi", gdi_h, gdi)
    start("wq", wq_h, wq)
    start("bx", bx_h.at[0], bxt)

    def chunk_copies(j):
        rows = pl.ds(j * CCH, CCH)
        return (pltpu.make_async_copy(wuk_h.at[rows], wuk.at[rows], sem.at[16 + 2 * j]),
                pltpu.make_async_copy(wuv_h.at[rows], wuv.at[rows], sem.at[17 + 2 * j]))

    for j in range(nch):
        for cp in chunk_copies(j):
            cp.start()
    start("ckv", ckv_h.at[0], ckv)
    start("wo", wo_h, wot)

    wait("ax", "fdt")
    RC = 512
    HR = -(-Df // 8) * 8
    for c0 in range(0, S, RC):
        x1t[:, c0:c0 + RC] = _dot(fdt[...], axt[:, c0:c0 + RC])

    for g in range(0, HR, 8):
        xs = [(x1t[g:g + 8, RB * a:RB * (a + 1)], x1t[HR + g:HR + g + 8, RB * a:RB * (a + 1)])
              for a in range(NB)]
        ys = _dft16(xs, -1)
        for k in range(NB):
            x1t[g:g + 8, RB * k:RB * (k + 1)] = ys[k][0]
            x1t[HR + g:HR + g + 8, RB * k:RB * (k + 1)] = ys[k][1]

    wait("wr", "wi", "gf", "gi")
    for src, dst in ((wrt, wrp), (wit, wip)):
        for j in range(0, RB, 32):
            v = src[:, j * NB:(j + 32) * NB].T.reshape(32, NB, Df)
            dst[:, j:j + 32, :] = jnp.swapaxes(v, 0, 1)

    for k1 in range(NB):
        rows = slice(k1 * RB, (k1 + 1) * RB)
        g = gf[k1]
        pr = _dot_nt(g, x1t[0:Df, rows].astype(_BF16))
        pi = _dot_nt(g, x1t[HR:HR + Df, rows].astype(_BF16))
        xr = pr[:RB] - pi[RB:]
        xi = pr[RB:] + pi[:RB]
        w_r = wrp[k1].astype(_F32)
        w_i = wip[k1].astype(_F32)
        yr = (xr * w_r - xi * w_i).astype(_BF16)
        yi = (xr * w_i + xi * w_r).astype(_BF16)
        h = gi[k1]
        qr = _dot(h, yr)
        qi = _dot(h, yi)
        zr[rows, :] = qr[:RB] + qi[RB:]
        zi[rows, :] = qi[:RB] - qr[RB:]

    for b0 in range(0, RB, 8):
        for (l0, l1) in ((0, 128), (128, Df)):
            xs = [(zr[RB * a + b0:RB * a + b0 + 8, l0:l1], zi[RB * a + b0:RB * a + b0 + 8, l0:l1])
                  for a in range(NB)]
            ys = _dft16(xs, +1)
            for k in range(NB):
                zr[RB * k + b0:RB * k + b0 + 8, l0:l1] = ys[k][0]
                zi[RB * k + b0:RB * k + b0 + 8, l0:l1] = ys[k][1]

    wait("gdr", "gdi")
    for r in range(0, S, RC):
        ya = _dot(zr[r:r + RC, :].astype(_BF16), gdr[...]) + _dot(zi[r:r + RC, :].astype(_BF16), gdi[...])
        stage[r:r + RC, 0:M] = ya.astype(_BF16)

    wait("wq", "bx")
    for c0 in range(0, S, RC):
        bx[c0:c0 + RC, :] = bxt[:, c0:c0 + RC].T
    for j in range(0, M, 64):
        wq_t[:, j:j + 64, :] = jnp.swapaxes(wq[j:j + 64], 0, 1)

    QR = 256
    DR = 16

    def qbody(j, c):
        jj = pl.multiple_of(j * CCH, CCH)

        def qtask(hh, r):
            def f():
                q_all[hh, r:r + QR, :] = _dot(bx[r:r + QR, :], wq_t[hh]).astype(_BF16)
            return f

        def dtask(src, lane0, u):
            def f():
                rows = pl.ds(pl.multiple_of(jj + u, DR), DR)
                wkv_t[:, rows, lane0:lane0 + D] = jnp.swapaxes(src[rows], 0, 1)
            return f

        for r in range(0, S, QR):
            qtask(2 * j, r)()
        for cp in chunk_copies(j):
            cp.wait()
        side = [dtask(src, l0, u) for u in range(0, CCH, DR) for (src, l0) in ((wuk, 0), (wuv, D))]
        _weave([qtask(2 * j + 1, r) for r in range(0, S, QR)], side)
        return c

    for j in range(nch):
        qbody(j, 0)

    wait("ckv")

    HS, HC, KR = S // 2, C // 2, 128
    for r in range(0, HS, KR):
        a11, a12 = ckv[r:r + KR, :HC].astype(_F32), ckv[r:r + KR, HC:].astype(_F32)
        a21, a22 = ckv[HS + r:HS + r + KR, :HC].astype(_F32), ckv[HS + r:HS + r + KR, HC:].astype(_F32)
        for i, v in enumerate((a11 + a22, a21 + a22, a11 + a12, a21 - a11, a12 - a22)):
            ac[i, r:r + KR, :] = v.astype(_BF16)

    def kv_proj_tasks(hh, slot):
        bc = {}

        def rhs():
            if not bc:
                def blk(i, j):
                    return jnp.concatenate(
                        [wkv_t[hh, i * HC:(i + 1) * HC, j * 128:(j + 1) * 128],
                         wkv_t[hh, i * HC:(i + 1) * HC, D + j * 128:D + (j + 1) * 128]], 1)
                b11, b12, b21, b22 = blk(0, 0), blk(0, 1), blk(1, 0), blk(1, 1)
                f11, f12, f21, f22 = (b.astype(_F32) for b in (b11, b12, b21, b22))
                bc.update(b1=(f11 + f22).astype(_BF16), b2=b11, b3=(f12 - f22).astype(_BF16),
                          b4=(f21 - f11).astype(_BF16), b5=b22, b6=(f11 + f12).astype(_BF16),
                          b7=(f21 + f22).astype(_BF16))
            return bc

        def task(r):
            def put(c, ro, j):
                c = c.astype(_BF16)
                kv[slot, ro:ro + KR, j * 128:(j + 1) * 128] = c[:, :128]
                kv[slot, ro:ro + KR, D + j * 128:D + (j + 1) * 128] = c[:, 128:]

            def f():
                b = rhs()
                m1 = _dot(ac[0, r:r + KR, :], b["b1"])
                m4 = _dot(ckv[HS + r:HS + r + KR, HC:], b["b4"])
                m5 = _dot(ac[2, r:r + KR, :], b["b5"])
                m7 = _dot(ac[4, r:r + KR, :], b["b7"])
                put(m1 + m4 - m5 + m7, r, 0)
                m3 = _dot(ckv[r:r + KR, :HC], b["b3"])
                put(m3 + m5, r, 1)
                m2 = _dot(ac[1, r:r + KR, :], b["b2"])
                put(m2 + m4, HS + r, 0)
                m6 = _dot(ac[3, r:r + KR, :], b["b6"])
                put(m1 - m2 + m3 + m6, HS + r, 1)
            return f

        return [task(r) for r in range(0, HS, KR)]

    for f in kv_proj_tasks(0, 0):
        f()
    wait("wo")
    acc[...] = jnp.zeros_like(acc)

    NQ = S // BQ
    SUB = 128
    nsub = BQ // SUB
    scale = _LOG2E * (D ** -0.5)

    def out_copy(i):
        return pltpu.make_async_copy(stage.at[pl.ds(i * BQ, BQ)], out_h.at[0, pl.ds(i * BQ, BQ)], osem.at[i])

    RH = 128
    order = list(range(NQ))[::-1]

    def head(h, last):
        slot = h % 2
        ls = {}

        def s_tasks(i, par):
            r0, r1 = i * BQ, (i + 1) * BQ
            ts = []
            for c0 in range(0, r0, BQ):
                def f(c0=c0):
                    sbuf[par, :, c0:c0 + BQ] = _dot_nt(q_all[h, r0:r1, :], kv[slot, c0:c0 + BQ, 0:D])
                ts.append(f)
            for t in range(nsub):
                def f(t=t):
                    c0 = r0 + t * SUB
                    sc = _dot_nt(q_all[h, c0:r1, :], kv[slot, c0:c0 + SUB, 0:D])
                    ri = lax.broadcasted_iota(jnp.int32, (SUB, SUB), 0)
                    ci = lax.broadcasted_iota(jnp.int32, (SUB, SUB), 1)
                    sbuf[par, t * SUB:(t + 1) * SUB, c0:c0 + SUB] = jnp.where(ci <= ri, sc[:SUB], _NEG)
                    if t + 1 < nsub:
                        sbuf[par, (t + 1) * SUB:, c0:c0 + SUB] = sc[SUB:]
                ts.append(f)
            return ts

        def sm_tasks(i, par):
            ts = []
            for j in range(BQ // RH):
                def f(j=j):
                    kvl = i * BQ + (j + 1) * RH
                    sc = sbuf[par, j * RH:(j + 1) * RH, 0:kvl]
                    m = jnp.max(sc, axis=1, keepdims=True)
                    p = jnp.exp2((sc - m) * scale)
                    ls[(i, j)] = jnp.sum(p, axis=1, keepdims=True)
                    pbuf[par, j * RH:(j + 1) * RH, 0:kvl] = p.astype(_BF16)
                ts.append(f)
            return ts

        def pv_tasks(i, par):
            ts = []
            for j in range(BQ // RH):
                def f(j=j):
                    kvl = i * BQ + (j + 1) * RH
                    o = _dot(pbuf[par, j * RH:(j + 1) * RH, 0:kvl], kv[slot, 0:kvl, D:2 * D])
                    cbuf[par, j * RH:(j + 1) * RH, :] = (o * (1.0 / ls[(i, j)])).astype(_BF16)
                ts.append(f)
            return ts

        def op_tasks(i, par):
            def f():
                r0, r1 = i * BQ, (i + 1) * BQ
                res = acc[:, r0:r1] + _dot_nt(wot[h], cbuf[par])
                if last:
                    stage[r0:r1, M:2 * M] = res.astype(_BF16).T
                    out_copy(i).start()
                else:
                    acc[:, r0:r1] = res
            return [f]

        kvt = [] if last else kv_proj_tasks(h + 1, 1 - slot)
        per = len(kvt) // NQ

        for f in s_tasks(order[0], 0):
            f()
        for n in range(NQ + 2):
            mx = s_tasks(order[n + 1], (n + 1) % 2) if n + 1 < NQ else []
            mx2 = []
            if 0 <= n - 2 < NQ:
                mx2 += op_tasks(order[n - 2], n % 2)
            if 0 <= n - 1 < NQ:
                mx2 += pv_tasks(order[n - 1], (n - 1) % 2)
            if n < NQ and not last:
                mx2 += kvt[n * per:(n + 1) * per]
            allm = []
            a = b = 0
            while a < len(mx) or b < len(mx2):
                if b >= len(mx2) or (a < len(mx) and a * len(mx2) <= b * len(mx)):
                    allm.append(mx[a])
                    a += 1
                else:
                    allm.append(mx2[b])
                    b += 1
            if n < NQ:
                _weave(sm_tasks(order[n], n % 2), allm)
            else:
                for f in allm:
                    f()

    def body(h, c):
        head(h, False)
        return c

    lax.fori_loop(0, H - 1, body, 0)
    head(H - 1, True)
    for i in range(NQ):
        out_copy(i).wait()


@jax.jit
def pallas_concat_heads__spectral_gfnet__compressed_kv_cla__prompt_kernel(
    A_x: jax.Array,
    A_w_r: jax.Array,
    A_w_i: jax.Array,
    B_x: jax.Array,
    B_c_kv: jax.Array,
    B_w_q: jax.Array,
    B_w_uk: jax.Array,
    B_w_uv: jax.Array,
    B_w_o: jax.Array,
):
    B, S, M = A_x.shape
    Df = M // 2 + 1
    C = B_c_kv.shape[-1]
    _, H, D = B_w_q.shape
    BQ = 512
    tables = [jnp.asarray(t) for t in _dft_tables(S, M)]

    vm = pltpu.VMEM
    HR = -(-Df // 8) * 8
    scratch = [
        vm((M, S), _BF16), vm((Df, S), _BF16), vm((Df, S), _BF16),
        vm((M, S), _BF16), vm((S, C), _BF16),
        vm((M, H, D), _BF16), vm((C, H, D), _BF16), vm((C, H, D), _BF16),
        vm((H, M, D), _BF16),
        vm((2 * HR, M), _BF16),
        vm((16, 256, 128), _BF16), vm((16, 256, 128), _BF16),
        vm((Df, M), _BF16), vm((Df, M), _BF16),
        vm((2 * HR, S), _F32), vm((S, Df), _F32), vm((S, Df), _F32),
        vm((16, S // 16, Df), _BF16), vm((16, S // 16, Df), _BF16),
        vm((S, M), _BF16),
        vm((H, M, D), _BF16), vm((H, C, 2 * D), _BF16),
        vm((H, S, D), _BF16), vm((2, S, 2 * D), _BF16),
        vm((M, S), _F32), vm((S, 2 * M), _BF16),
        vm((2, BQ, S), _F32), vm((2, BQ, S), _BF16), vm((2, BQ, D), _BF16),
        vm((5, S // 2, C // 2), _BF16),
        pltpu.SemaphoreType.DMA((16 + 2 * (C // 128),)),
        pltpu.SemaphoreType.DMA((S // BQ,)),
    ]
    any_spec = pl.BlockSpec(memory_space=pltpu.HBM)
    return pl.pallas_call(
        functools.partial(_kernel, S=S, M=M, H=H, D=D, C=C, BQ=BQ),
        in_specs=[any_spec] * 14,
        out_specs=any_spec,
        out_shape=jax.ShapeDtypeStruct((B, S, 2 * M), _BF16),
        scratch_shapes=scratch,
        compiler_params=pltpu.CompilerParams(vmem_limit_bytes=120 * 2**20),
        name="gfnet_cla",
    )(jnp.swapaxes(A_x, 1, 2), A_w_r.T, A_w_i.T, jnp.swapaxes(B_x, 1, 2), B_c_kv,
      B_w_q, B_w_uk, B_w_uv, jnp.swapaxes(B_w_o, 1, 2), *tables)
```

```python
import functools

import jax
import jax.numpy as jnp
import numpy as np
from jax import lax
import jax.experimental.pallas as pl
import jax.experimental.pallas.tpu as pltpu

_BF16 = jnp.bfloat16
_F32 = jnp.float32
_NT = (((1,), (1,)), ((), ()))
_LOG2E = 1.4426950408889634
_NEG = -1e30


def _np_bf16(a):
    import ml_dtypes
    return np.asarray(a, np.float64).astype(np.float32).astype(ml_dtypes.bfloat16)


@functools.lru_cache(maxsize=None)
def _dft_tables(S, D):
    Df = D // 2 + 1
    n1, n2 = 16, S // 16
    d = np.arange(D)[:, None]
    c = np.arange(Df)[None, :]
    ang = 2.0 * np.pi * ((d * c) % D) / D
    fdr = np.cos(ang)
    fdi = -np.sin(ang)
    wgt = np.full(Df, 2.0)
    wgt[0] = 1.0
    if D % 2 == 0:
        wgt[-1] = 1.0
    gdr = wgt[:, None] * np.cos(ang.T) / (S * D)
    gdi = -wgt[:, None] * np.sin(ang.T) / (S * D)
    k1 = np.arange(n1)[:, None, None]
    k2 = np.arange(n2)[None, :, None]
    b = np.arange(n2)[None, None, :]
    g = np.exp(-2j * np.pi * ((b * (k1 + n1 * k2)) % S) / S)
    gf = np.concatenate([g.real, g.imag], axis=1)
    gt = np.transpose(g, (0, 2, 1))
    gi = np.concatenate([gt.real, gt.imag], axis=1)
    hr = -(-Df // 8) * 8
    fdt = np.zeros((2 * hr, D))
    fdt[:Df] = fdr.T
    fdt[hr:hr + Df] = fdi.T
    return tuple(_np_bf16(t) for t in (fdt, gf, gi, gdr, gdi))


_R2 = float(np.sqrt(0.5))
_C1, _S1 = float(np.cos(np.pi / 8)), float(np.sin(np.pi / 8))


def _cmul(ar, ai, wr, wi):
    return ar * wr - ai * wi, ar * wi + ai * wr


def _tw16(ar, ai, e, sign):
    e %= 16
    if e == 0:
        return ar, ai
    if e == 4:
        return (-ai, ar) if sign > 0 else (ai, -ar)
    if e == 2:
        return ((ar - ai) * _R2, (ar + ai) * _R2) if sign > 0 else ((ar + ai) * _R2, (ai - ar) * _R2)
    if e == 6:
        return ((-ar - ai) * _R2, (ar - ai) * _R2) if sign > 0 else ((ai - ar) * _R2, (-ar - ai) * _R2)
    ang = sign * 2.0 * np.pi * e / 16
    return _cmul(ar, ai, float(np.cos(ang)), float(np.sin(ang)))


def _dft4(x, sign):
    (ar, ai), (br, bi), (cr, ci), (dr, di) = x
    t0r, t0i = ar + cr, ai + ci
    t1r, t1i = ar - cr, ai - ci
    t2r, t2i = br + dr, bi + di
    t3r, t3i = br - dr, bi - di
    y0 = (t0r + t2r, t0i + t2i)
    y2 = (t0r - t2r, t0i - t2i)
    if sign < 0:
        y1 = (t1r + t3i, t1i - t3r)
        y3 = (t1r - t3i, t1i + t3r)
    else:
        y1 = (t1r - t3i, t1i + t3r)
        y3 = (t1r + t3i, t1i - t3r)
    return [y0, y1, y2, y3]


def _dft16(x, sign):
    cols = []
    for n2 in range(4):
        y = _dft4([x[4 * n1 + n2] for n1 in range(4)], sign)
        cols.append([_tw16(y[k1][0], y[k1][1], n2 * k1, sign) for k1 in range(4)])
    out = [None] * 16
    for k1 in range(4):
        z = _dft4([cols[n2][k1] for n2 in range(4)], sign)
        for k2 in range(4):
            out[k1 + 4 * k2] = z[k2]
    return out


def _dot(a, b):
    return jnp.dot(a, b, preferred_element_type=_F32)


def _dot_nt(a, b):
    return lax.dot_general(a, b, _NT, preferred_element_type=_F32)


def _weave(main, side):
    k = 0
    for j, f in enumerate(main):
        f()
        upto = len(side) * (j + 1) // len(main)
        while k < upto:
            side[k]()
            k += 1
    for f in side[k:]:
        f()


def _kernel(ax_h, wr_h, wi_h, bx_h, ckv_h, wq_h, wuk_h, wuv_h, wo_h,
            fdt_h, gf_h, gi_h, gdr_h, gdi_h, zero_ref,
            out_h,
            axt, wrt, wit, bxt, ckv, wq, wuk, wuv, wot, fdt, gf, gi, gdr, gdi,
            x1t, zr, zi, wrp, wip, bx,
            wq_t, wkv_t, q_all, kv, acc, stage, sbuf, pbuf, cbuf, ac, sem, osem,
            *, S, M, H, D, C, BQ):
    Df = M // 2 + 1
    NB = 16
    RB = S // NB
    CCH = 128
    nch = C // CCH

    copies = {}
    sem_ids = {}

    def start(name, src, dst):
        i = len(sem_ids)
        sem_ids[name] = i
        cp = pltpu.make_async_copy(src, dst, sem.at[i])
        cp.start()
        copies[name] = cp

    def wait(*names):
        for n in names:
            copies[n].wait()

    start("ax", ax_h.at[0], axt)
    start("fdt", fdt_h, fdt)
    start("gf", gf_h, gf)
    start("wr", wr_h, wrt)
    start("wi", wi_h, wit)
    start("gi", gi_h, gi)
    start("gdr", gdr_h, gdr)
    start("gdi", gdi_h, gdi)
    start("wq", wq_h, wq)
    start("bx", bx_h.at[0], bxt)

    def chunk_copies(j):
        rows = pl.ds(j * CCH, CCH)
        return (pltpu.make_async_copy(wuk_h.at[rows], wuk.at[rows], sem.at[16 + 2 * j]),
                pltpu.make_async_copy(wuv_h.at[rows], wuv.at[rows], sem.at[17 + 2 * j]))

    for j in range(nch):
        for cp in chunk_copies(j):
            cp.start()
    start("ckv", ckv_h.at[0], ckv)
    start("wo", wo_h, wot)

    wait("ax", "fdt")
    RC = 512
    HR = -(-Df // 8) * 8
    for c0 in range(0, S, RC):
        x1t[:, c0:c0 + RC] = _dot(fdt[...], axt[:, c0:c0 + RC])

    for g in range(0, HR, 8):
        xs = [(x1t[g:g + 8, RB * a:RB * (a + 1)], x1t[HR + g:HR + g + 8, RB * a:RB * (a + 1)])
              for a in range(NB)]
        ys = _dft16(xs, -1)
        for k in range(NB):
            x1t[g:g + 8, RB * k:RB * (k + 1)] = ys[k][0]
            x1t[HR + g:HR + g + 8, RB * k:RB * (k + 1)] = ys[k][1]

    wait("wr", "wi", "gf", "gi")
    for src, dst in ((wrt, wrp), (wit, wip)):
        for j in range(0, RB, 32):
            v = src[:, j * NB:(j + 32) * NB].T.reshape(32, NB, Df)
            dst[:, j:j + 32, :] = jnp.swapaxes(v, 0, 1)

    for k1 in range(NB):
        rows = slice(k1 * RB, (k1 + 1) * RB)
        g = gf[k1]
        pr = _dot_nt(g, x1t[0:Df, rows].astype(_BF16))
        pi = _dot_nt(g, x1t[HR:HR + Df, rows].astype(_BF16))
        xr = pr[:RB] - pi[RB:]
        xi = pr[RB:] + pi[:RB]
        w_r = wrp[k1].astype(_F32)
        w_i = wip[k1].astype(_F32)
        yr = (xr * w_r - xi * w_i).astype(_BF16)
        yi = (xr * w_i + xi * w_r).astype(_BF16)
        h = gi[k1]
        qr = _dot(h, yr)
        qi = _dot(h, yi)
        zr[rows, :] = qr[:RB] + qi[RB:]
        zi[rows, :] = qi[:RB] - qr[RB:]

    for b0 in range(0, RB, 8):
        for (l0, l1) in ((0, 128), (128, Df)):
            xs = [(zr[RB * a + b0:RB * a + b0 + 8, l0:l1], zi[RB * a + b0:RB * a + b0 + 8, l0:l1])
                  for a in range(NB)]
            ys = _dft16(xs, +1)
            for k in range(NB):
                zr[RB * k + b0:RB * k + b0 + 8, l0:l1] = ys[k][0]
                zi[RB * k + b0:RB * k + b0 + 8, l0:l1] = ys[k][1]

    wait("gdr", "gdi")
    for r in range(0, S, RC):
        ya = _dot(zr[r:r + RC, :].astype(_BF16), gdr[...]) + _dot(zi[r:r + RC, :].astype(_BF16), gdi[...])
        stage[r:r + RC, 0:M] = ya.astype(_BF16)

    wait("wq", "bx")
    for c0 in range(0, S, RC):
        bx[c0:c0 + RC, :] = bxt[:, c0:c0 + RC].T
    for j in range(0, M, 64):
        wq_t[:, j:j + 64, :] = jnp.swapaxes(wq[j:j + 64], 0, 1)

    never = zero_ref[0] != 0
    pending = []

    def after_pending(lhs):
        if not pending:
            return lhs
        t = lhs[:16, :128]
        while pending:
            t = jnp.where(never, pending.pop(), t)
        return jnp.concatenate([jnp.concatenate([t, lhs[:16, 128:]], 1), lhs[16:]], 0)

    QR = 256
    DR = 16

    def qbody(j, c):
        jj = pl.multiple_of(j * CCH, CCH)

        def qtask(hh, r):
            def f():
                q_all[hh, r:r + QR, :] = _dot(after_pending(bx[r:r + QR, :]), wq_t[hh]).astype(_BF16)
            return f

        def dtask(src, lane0, u):
            def f():
                rows = pl.ds(pl.multiple_of(jj + u, DR), DR)
                v = jnp.swapaxes(src[rows], 0, 1)
                wkv_t[:, rows, lane0:lane0 + D] = v
                pending.extend([v[0, :16, :128], v[0, :16, 128:]])
            return f

        for cp in chunk_copies(j):
            cp.wait()
        side = [dtask(src, l0, u) for u in range(0, CCH, DR) for (src, l0) in ((wuk, 0), (wuv, D))]
        _weave([qtask(2 * j + t, r) for t in range(2) for r in range(0, S, QR)], side)
        return c

    for j in range(nch):
        qbody(j, 0)

    wait("ckv")

    HS, HC, KR = S // 2, C // 2, 128
    for r in range(0, HS, KR):
        a11, a12 = ckv[r:r + KR, :HC].astype(_F32), ckv[r:r + KR, HC:].astype(_F32)
        a21, a22 = ckv[HS + r:HS + r + KR, :HC].astype(_F32), ckv[HS + r:HS + r + KR, HC:].astype(_F32)
        for i, v in enumerate((a11 + a22, a21 + a22, a11 + a12, a21 - a11, a12 - a22)):
            ac[i, r:r + KR, :] = v.astype(_BF16)

    def kv_proj_tasks(hh, slot):
        bc = {}

        def rhs():
            if not bc:
                def blk(i, j):
                    return jnp.concatenate(
                        [wkv_t[hh, i * HC:(i + 1) * HC, j * 128:(j + 1) * 128],
                         wkv_t[hh, i * HC:(i + 1) * HC, D + j * 128:D + (j + 1) * 128]], 1)
                b11, b12, b21, b22 = blk(0, 0), blk(0, 1), blk(1, 0), blk(1, 1)
                f11, f12, f21, f22 = (b.astype(_F32) for b in (b11, b12, b21, b22))
                bc.update(b1=(f11 + f22).astype(_BF16), b2=b11, b3=(f12 - f22).astype(_BF16),
                          b4=(f21 - f11).astype(_BF16), b5=b22, b6=(f11 + f12).astype(_BF16),
                          b7=(f21 + f22).astype(_BF16))
            return bc

        def task(r):
            def put(c, ro, j):
                c = c.astype(_BF16)
                kv[slot, ro:ro + KR, j * 128:(j + 1) * 128] = c[:, :128]
                kv[slot, ro:ro + KR, D + j * 128:D + (j + 1) * 128] = c[:, 128:]

            def f():
                b = rhs()
                m1 = _dot(ac[0, r:r + KR, :], b["b1"])
                m4 = _dot(ckv[HS + r:HS + r + KR, HC:], b["b4"])
                m5 = _dot(ac[2, r:r + KR, :], b["b5"])
                m7 = _dot(ac[4, r:r + KR, :], b["b7"])
                put(m1 + m4 - m5 + m7, r, 0)
                m3 = _dot(ckv[r:r + KR, :HC], b["b3"])
                put(m3 + m5, r, 1)
                m2 = _dot(ac[1, r:r + KR, :], b["b2"])
                put(m2 + m4, HS + r, 0)
                m6 = _dot(ac[3, r:r + KR, :], b["b6"])
                put(m1 - m2 + m3 + m6, HS + r, 1)
            return f

        return [task(r) for r in range(0, HS, KR)]

    for f in kv_proj_tasks(0, 0):
        f()
    wait("wo")
    acc[...] = jnp.zeros_like(acc)

    NQ = S // BQ
    SUB = 128
    nsub = BQ // SUB
    scale = _LOG2E * (D ** -0.5)

    def out_copy(i):
        return pltpu.make_async_copy(stage.at[pl.ds(i * BQ, BQ)], out_h.at[0, pl.ds(i * BQ, BQ)], osem.at[i])

    RH = 128
    order = list(range(NQ))[::-1]

    def head(h, last):
        slot = h % 2
        ls = {}

        def s_tasks(i, par):
            r0, r1 = i * BQ, (i + 1) * BQ
            ts = []
            for c0 in range(0, r0, BQ):
                def f(c0=c0):
                    sbuf[par, :, c0:c0 + BQ] = _dot_nt(q_all[h, r0:r1, :], kv[slot, c0:c0 + BQ, 0:D])
                ts.append(f)
            for t in range(nsub):
                def f(t=t):
                    c0 = r0 + t * SUB
                    sc = _dot_nt(q_all[h, c0:r1, :], kv[slot, c0:c0 + SUB, 0:D])
                    ri = lax.broadcasted_iota(jnp.int32, (SUB, SUB), 0)
                    ci = lax.broadcasted_iota(jnp.int32, (SUB, SUB), 1)
                    sbuf[par, t * SUB:(t + 1) * SUB, c0:c0 + SUB] = jnp.where(ci <= ri, sc[:SUB], _NEG)
                    if t + 1 < nsub:
                        sbuf[par, (t + 1) * SUB:, c0:c0 + SUB] = sc[SUB:]
                ts.append(f)
            return ts

        def sm_tasks(i, par):
            ts = []
            for j in range(BQ // RH):
                def f(j=j):
                    kvl = i * BQ + (j + 1) * RH
                    sc = sbuf[par, j * RH:(j + 1) * RH, 0:kvl]
                    m = jnp.max(sc, axis=1, keepdims=True)
                    p = jnp.exp2((sc - m) * scale)
                    ls[(i, j)] = jnp.sum(p, axis=1, keepdims=True)
                    pbuf[par, j * RH:(j + 1) * RH, 0:kvl] = p.astype(_BF16)
                ts.append(f)
            return ts

        def pv_tasks(i, par):
            ts = []
            for j in range(BQ // RH):
                def f(j=j):
                    kvl = i * BQ + (j + 1) * RH
                    o = _dot(pbuf[par, j * RH:(j + 1) * RH, 0:kvl], kv[slot, 0:kvl, D:2 * D])
                    cbuf[par, j * RH:(j + 1) * RH, :] = (o * (1.0 / ls[(i, j)])).astype(_BF16)
                ts.append(f)
            return ts

        def op_tasks(i, par):
            def f():
                r0, r1 = i * BQ, (i + 1) * BQ
                res = acc[:, r0:r1] + _dot_nt(wot[h], cbuf[par])
                if last:
                    stage[r0:r1, M:2 * M] = res.astype(_BF16).T
                    out_copy(i).start()
                else:
                    acc[:, r0:r1] = res
            return [f]

        kvt = [] if last else kv_proj_tasks(h + 1, 1 - slot)
        per = len(kvt) // NQ

        for f in s_tasks(order[0], 0):
            f()
        for n in range(NQ + 2):
            mx = s_tasks(order[n + 1], (n + 1) % 2) if n + 1 < NQ else []
            mx2 = []
            if 0 <= n - 2 < NQ:
                mx2 += op_tasks(order[n - 2], n % 2)
            if 0 <= n - 1 < NQ:
                mx2 += pv_tasks(order[n - 1], (n - 1) % 2)
            if n < NQ and not last:
                mx2 += kvt[n * per:(n + 1) * per]
            allm = []
            a = b = 0
            while a < len(mx) or b < len(mx2):
                if b >= len(mx2) or (a < len(mx) and a * len(mx2) <= b * len(mx)):
                    allm.append(mx[a])
                    a += 1
                else:
                    allm.append(mx2[b])
                    b += 1
            if n < NQ:
                _weave(sm_tasks(order[n], n % 2), allm)
            else:
                for f in allm:
                    f()

    def body(h, c):
        head(h, False)
        return c

    lax.fori_loop(0, H - 1, body, 0)
    head(H - 1, True)
    for i in range(NQ):
        out_copy(i).wait()


@jax.jit
def pallas_concat_heads__spectral_gfnet__compressed_kv_cla__prompt_kernel(
    A_x: jax.Array,
    A_w_r: jax.Array,
    A_w_i: jax.Array,
    B_x: jax.Array,
    B_c_kv: jax.Array,
    B_w_q: jax.Array,
    B_w_uk: jax.Array,
    B_w_uv: jax.Array,
    B_w_o: jax.Array,
):
    B, S, M = A_x.shape
    Df = M // 2 + 1
    C = B_c_kv.shape[-1]
    _, H, D = B_w_q.shape
    BQ = 512
    tables = [jnp.asarray(t) for t in _dft_tables(S, M)]

    vm = pltpu.VMEM
    HR = -(-Df // 8) * 8
    scratch = [
        vm((M, S), _BF16), vm((Df, S), _BF16), vm((Df, S), _BF16),
        vm((M, S), _BF16), vm((S, C), _BF16),
        vm((M, H, D), _BF16), vm((C, H, D), _BF16), vm((C, H, D), _BF16),
        vm((H, M, D), _BF16),
        vm((2 * HR, M), _BF16),
        vm((16, 256, 128), _BF16), vm((16, 256, 128), _BF16),
        vm((Df, M), _BF16), vm((Df, M), _BF16),
        vm((2 * HR, S), _F32), vm((S, Df), _F32), vm((S, Df), _F32),
        vm((16, S // 16, Df), _BF16), vm((16, S // 16, Df), _BF16),
        vm((S, M), _BF16),
        vm((H, M, D), _BF16), vm((H, C, 2 * D), _BF16),
        vm((H, S, D), _BF16), vm((2, S, 2 * D), _BF16),
        vm((M, S), _F32), vm((S, 2 * M), _BF16),
        vm((2, BQ, S), _F32), vm((2, BQ, S), _BF16), vm((2, BQ, D), _BF16),
        vm((5, S // 2, C // 2), _BF16),
        pltpu.SemaphoreType.DMA((16 + 2 * (C // 128),)),
        pltpu.SemaphoreType.DMA((S // BQ,)),
    ]
    any_spec = pl.BlockSpec(memory_space=pltpu.HBM)
    return pl.pallas_call(
        functools.partial(_kernel, S=S, M=M, H=H, D=D, C=C, BQ=BQ),
        in_specs=[any_spec] * 14 + [pl.BlockSpec(memory_space=pltpu.SMEM)],
        out_specs=any_spec,
        out_shape=jax.ShapeDtypeStruct((B, S, 2 * M), _BF16),
        scratch_shapes=scratch,
        compiler_params=pltpu.CompilerParams(vmem_limit_bytes=120 * 2**20),
        name="gfnet_cla",
    )(jnp.swapaxes(A_x, 1, 2), A_w_r.T, A_w_i.T, jnp.swapaxes(B_x, 1, 2), B_c_kv,
      B_w_q, B_w_uk, B_w_uv, jnp.swapaxes(B_w_o, 1, 2), *tables, jnp.asarray(np.zeros((1,), np.int32)))
```

```python
import functools

import jax
import jax.numpy as jnp
import numpy as np
from jax import lax
import jax.experimental.pallas as pl
import jax.experimental.pallas.tpu as pltpu

_BF16 = jnp.bfloat16
_F32 = jnp.float32
_NT = (((1,), (1,)), ((), ()))
_LOG2E = 1.4426950408889634
_NEG = -1e30


def _np_bf16(a):
    import ml_dtypes
    return np.asarray(a, np.float64).astype(np.float32).astype(ml_dtypes.bfloat16)


@functools.lru_cache(maxsize=None)
def _dft_tables(S, D):
    Df = D // 2 + 1
    n1, n2 = 16, S // 16
    d = np.arange(D)[:, None]
    c = np.arange(Df)[None, :]
    ang = 2.0 * np.pi * ((d * c) % D) / D
    fdr = np.cos(ang)
    fdi = -np.sin(ang)
    wgt = np.full(Df, 2.0)
    wgt[0] = 1.0
    if D % 2 == 0:
        wgt[-1] = 1.0
    gdr = wgt[:, None] * np.cos(ang.T) / (S * D)
    gdi = -wgt[:, None] * np.sin(ang.T) / (S * D)
    k1 = np.arange(n1)[:, None, None]
    k2 = np.arange(n2)[None, :, None]
    b = np.arange(n2)[None, None, :]
    g = np.exp(-2j * np.pi * ((b * (k1 + n1 * k2)) % S) / S)
    gf = np.concatenate([g.real, g.imag], axis=1)
    gt = np.transpose(g, (0, 2, 1))
    gi = np.concatenate([gt.real, gt.imag], axis=1)
    hr = -(-Df // 8) * 8
    fdt = np.zeros((2 * hr, D))
    fdt[:Df] = fdr.T
    fdt[hr:hr + Df] = fdi.T
    return tuple(_np_bf16(t) for t in (fdt, gf, gi, gdr, gdi))


_R2 = float(np.sqrt(0.5))
_C1, _S1 = float(np.cos(np.pi / 8)), float(np.sin(np.pi / 8))


def _cmul(ar, ai, wr, wi):
    return ar * wr - ai * wi, ar * wi + ai * wr


def _tw16(ar, ai, e, sign):
    e %= 16
    if e == 0:
        return ar, ai
    if e == 4:
        return (-ai, ar) if sign > 0 else (ai, -ar)
    if e == 2:
        return ((ar - ai) * _R2, (ar + ai) * _R2) if sign > 0 else ((ar + ai) * _R2, (ai - ar) * _R2)
    if e == 6:
        return ((-ar - ai) * _R2, (ar - ai) * _R2) if sign > 0 else ((ai - ar) * _R2, (-ar - ai) * _R2)
    ang = sign * 2.0 * np.pi * e / 16
    return _cmul(ar, ai, float(np.cos(ang)), float(np.sin(ang)))


def _dft4(x, sign):
    (ar, ai), (br, bi), (cr, ci), (dr, di) = x
    t0r, t0i = ar + cr, ai + ci
    t1r, t1i = ar - cr, ai - ci
    t2r, t2i = br + dr, bi + di
    t3r, t3i = br - dr, bi - di
    y0 = (t0r + t2r, t0i + t2i)
    y2 = (t0r - t2r, t0i - t2i)
    if sign < 0:
        y1 = (t1r + t3i, t1i - t3r)
        y3 = (t1r - t3i, t1i + t3r)
    else:
        y1 = (t1r - t3i, t1i + t3r)
        y3 = (t1r + t3i, t1i - t3r)
    return [y0, y1, y2, y3]


def _dft16(x, sign):
    cols = []
    for n2 in range(4):
        y = _dft4([x[4 * n1 + n2] for n1 in range(4)], sign)
        cols.append([_tw16(y[k1][0], y[k1][1], n2 * k1, sign) for k1 in range(4)])
    out = [None] * 16
    for k1 in range(4):
        z = _dft4([cols[n2][k1] for n2 in range(4)], sign)
        for k2 in range(4):
            out[k1 + 4 * k2] = z[k2]
    return out


def _dot(a, b):
    return jnp.dot(a, b, preferred_element_type=_F32)


def _dot_nt(a, b):
    return lax.dot_general(a, b, _NT, preferred_element_type=_F32)


def _weave(main, side):
    k = 0
    for j, f in enumerate(main):
        f()
        upto = len(side) * (j + 1) // len(main)
        while k < upto:
            side[k]()
            k += 1
    for f in side[k:]:
        f()


def _kernel(ax_h, wr_h, wi_h, bx_h, ckv_h, wq_h, wuk_h, wuv_h, wo_h,
            fdt_h, gf_h, gi_h, gdr_h, gdi_h, zero_ref,
            out_h,
            axt, wrt, wit, bxt, ckv, wq, wuk, wuv, wot, fdt, gf, gi, gdr, gdi,
            x1t, zr, zi, wrp, wip, bx,
            wq_t, wkv_t, q_all, kv, acc, stage, sbuf, pbuf, cbuf, ac, sem, osem,
            *, S, M, H, D, C, BQ):
    Df = M // 2 + 1
    NB = 16
    RB = S // NB
    CCH = 128
    nch = C // CCH

    copies = {}
    sem_ids = {}

    def start(name, src, dst):
        i = len(sem_ids)
        sem_ids[name] = i
        cp = pltpu.make_async_copy(src, dst, sem.at[i])
        cp.start()
        copies[name] = cp

    def wait(*names):
        for n in names:
            copies[n].wait()

    start("ax", ax_h.at[0], axt)
    start("fdt", fdt_h, fdt)
    start("gf", gf_h, gf)
    start("wr", wr_h, wrt)
    start("wi", wi_h, wit)
    start("gi", gi_h, gi)
    start("gdr", gdr_h, gdr)
    start("gdi", gdi_h, gdi)
    start("wq", wq_h, wq)
    start("bx", bx_h.at[0], bxt)

    def chunk_copies(j):
        rows = pl.ds(j * CCH, CCH)
        return (pltpu.make_async_copy(wuk_h.at[rows], wuk.at[rows], sem.at[16 + 2 * j]),
                pltpu.make_async_copy(wuv_h.at[rows], wuv.at[rows], sem.at[17 + 2 * j]))

    for j in range(nch):
        for cp in chunk_copies(j):
            cp.start()
    start("ckv", ckv_h.at[0], ckv)
    start("wo", wo_h, wot)

    wait("ax", "fdt")
    RC = 512
    HR = -(-Df // 8) * 8
    for c0 in range(0, S, RC):
        x1t[:, c0:c0 + RC] = _dot(fdt[...], axt[:, c0:c0 + RC])

    for g in range(0, HR, 8):
        xs = [(x1t[g:g + 8, RB * a:RB * (a + 1)], x1t[HR + g:HR + g + 8, RB * a:RB * (a + 1)])
              for a in range(NB)]
        ys = _dft16(xs, -1)
        for k in range(NB):
            x1t[g:g + 8, RB * k:RB * (k + 1)] = ys[k][0]
            x1t[HR + g:HR + g + 8, RB * k:RB * (k + 1)] = ys[k][1]

    wait("wr", "wi", "gf", "gi")
    for src, dst in ((wrt, wrp), (wit, wip)):
        for j in range(0, RB, 32):
            v = src[:, j * NB:(j + 32) * NB].T.reshape(32, NB, Df)
            dst[:, j:j + 32, :] = jnp.swapaxes(v, 0, 1)

    def fwd(k1):
        rows = slice(k1 * RB, (k1 + 1) * RB)
        g = gf[k1]
        pr = _dot_nt(g, x1t[0:Df, rows].astype(_BF16))
        pi = _dot_nt(g, x1t[HR:HR + Df, rows].astype(_BF16))
        return pr[:RB] - pi[RB:], pr[RB:] + pi[:RB]

    nxt = fwd(0)
    for k1 in range(NB):
        rows = slice(k1 * RB, (k1 + 1) * RB)
        xr, xi = nxt
        if k1 + 1 < NB:
            nxt = fwd(k1 + 1)
        w_r = wrp[k1].astype(_F32)
        w_i = wip[k1].astype(_F32)
        yr = (xr * w_r - xi * w_i).astype(_BF16)
        yi = (xr * w_i + xi * w_r).astype(_BF16)
        h = gi[k1]
        qr = _dot(h, yr)
        qi = _dot(h, yi)
        zr[rows, :] = qr[:RB] + qi[RB:]
        zi[rows, :] = qi[:RB] - qr[RB:]

    for b0 in range(0, RB, 8):
        for (l0, l1) in ((0, 128), (128, Df)):
            xs = [(zr[RB * a + b0:RB * a + b0 + 8, l0:l1], zi[RB * a + b0:RB * a + b0 + 8, l0:l1])
                  for a in range(NB)]
            ys = _dft16(xs, +1)
            for k in range(NB):
                zr[RB * k + b0:RB * k + b0 + 8, l0:l1] = ys[k][0]
                zi[RB * k + b0:RB * k + b0 + 8, l0:l1] = ys[k][1]

    wait("gdr", "gdi")
    for r in range(0, S, RC):
        ya = _dot(zr[r:r + RC, :].astype(_BF16), gdr[...]) + _dot(zi[r:r + RC, :].astype(_BF16), gdi[...])
        stage[r:r + RC, 0:M] = ya.astype(_BF16)

    wait("wq", "bx")
    for c0 in range(0, S, RC):
        bx[c0:c0 + RC, :] = bxt[:, c0:c0 + RC].T
    for j in range(0, M, 64):
        wq_t[:, j:j + 64, :] = jnp.swapaxes(wq[j:j + 64], 0, 1)

    never = zero_ref[0] != 0
    pending = []

    def after_pending(lhs):
        if not pending:
            return lhs
        t = lhs[:16, :128]
        while pending:
            t = jnp.where(never, pending.pop(), t)
        return jnp.concatenate([jnp.concatenate([t, lhs[:16, 128:]], 1), lhs[16:]], 0)

    QR = 256
    DR = 16

    def qbody(j, c):
        jj = pl.multiple_of(j * CCH, CCH)

        def qtask(hh, r):
            def f():
                q_all[hh, r:r + QR, :] = _dot(after_pending(bx[r:r + QR, :]), wq_t[hh]).astype(_BF16)
            return f

        def dtask(src, lane0, u):
            def f():
                rows = pl.ds(pl.multiple_of(jj + u, DR), DR)
                v = jnp.swapaxes(src[rows], 0, 1)
                wkv_t[:, rows, lane0:lane0 + D] = v
                pending.extend([v[0, :16, :128], v[0, :16, 128:]])
            return f

        for cp in chunk_copies(j):
            cp.wait()
        side = [dtask(src, l0, u) for u in range(0, CCH, DR) for (src, l0) in ((wuk, 0), (wuv, D))]
        _weave([qtask(2 * j + t, r) for t in range(2) for r in range(0, S, QR)], side)
        return c

    for j in range(nch):
        qbody(j, 0)

    wait("ckv")

    HS, HC, KR = S // 2, C // 2, 128
    for r in range(0, HS, KR):
        a11, a12 = ckv[r:r + KR, :HC].astype(_F32), ckv[r:r + KR, HC:].astype(_F32)
        a21, a22 = ckv[HS + r:HS + r + KR, :HC].astype(_F32), ckv[HS + r:HS + r + KR, HC:].astype(_F32)
        for i, v in enumerate((a11 + a22, a21 + a22, a11 + a12, a21 - a11, a12 - a22)):
            ac[i, r:r + KR, :] = v.astype(_BF16)

    def kv_proj_tasks(hh, slot):
        bc = {}

        def rhs():
            if not bc:
                def blk(i, j):
                    return jnp.concatenate(
                        [wkv_t[hh, i * HC:(i + 1) * HC, j * 128:(j + 1) * 128],
                         wkv_t[hh, i * HC:(i + 1) * HC, D + j * 128:D + (j + 1) * 128]], 1)
                b11, b12, b21, b22 = blk(0, 0), blk(0, 1), blk(1, 0), blk(1, 1)
                f11, f12, f21, f22 = (b.astype(_F32) for b in (b11, b12, b21, b22))
                bc.update(b1=(f11 + f22).astype(_BF16), b2=b11, b3=(f12 - f22).astype(_BF16),
                          b4=(f21 - f11).astype(_BF16), b5=b22, b6=(f11 + f12).astype(_BF16),
                          b7=(f21 + f22).astype(_BF16))
            return bc

        def task(r):
            def put(c, ro, j):
                c = c.astype(_BF16)
                kv[slot, ro:ro + KR, j * 128:(j + 1) * 128] = c[:, :128]
                kv[slot, ro:ro + KR, D + j * 128:D + (j + 1) * 128] = c[:, 128:]

            def f():
                b = rhs()
                m1 = _dot(ac[0, r:r + KR, :], b["b1"])
                m4 = _dot(ckv[HS + r:HS + r + KR, HC:], b["b4"])
                m5 = _dot(ac[2, r:r + KR, :], b["b5"])
                m7 = _dot(ac[4, r:r + KR, :], b["b7"])
                put(m1 + m4 - m5 + m7, r, 0)
                m3 = _dot(ckv[r:r + KR, :HC], b["b3"])
                put(m3 + m5, r, 1)
                m2 = _dot(ac[1, r:r + KR, :], b["b2"])
                put(m2 + m4, HS + r, 0)
                m6 = _dot(ac[3, r:r + KR, :], b["b6"])
                put(m1 - m2 + m3 + m6, HS + r, 1)
            return f

        return [task(r) for r in range(0, HS, KR)]

    for f in kv_proj_tasks(0, 0):
        f()
    wait("wo")
    acc[...] = jnp.zeros_like(acc)

    NQ = S // BQ
    SUB = 128
    nsub = BQ // SUB
    scale = _LOG2E * (D ** -0.5)

    def out_copy(i):
        return pltpu.make_async_copy(stage.at[pl.ds(i * BQ, BQ)], out_h.at[0, pl.ds(i * BQ, BQ)], osem.at[i])

    RH = 128
    order = list(range(NQ))[::-1]

    def head(h, last):
        slot = h % 2
        ls = {}

        def s_tasks(i, par):
            r0, r1 = i * BQ, (i + 1) * BQ
            ts = []
            for c0 in range(0, r0, BQ):
                def f(c0=c0):
                    sbuf[par, :, c0:c0 + BQ] = _dot_nt(q_all[h, r0:r1, :], kv[slot, c0:c0 + BQ, 0:D])
                ts.append(f)
            for t in range(nsub):
                def f(t=t):
                    c0 = r0 + t * SUB
                    sc = _dot_nt(q_all[h, c0:r1, :], kv[slot, c0:c0 + SUB, 0:D])
                    ri = lax.broadcasted_iota(jnp.int32, (SUB, SUB), 0)
                    ci = lax.broadcasted_iota(jnp.int32, (SUB, SUB), 1)
                    sbuf[par, t * SUB:(t + 1) * SUB, c0:c0 + SUB] = jnp.where(ci <= ri, sc[:SUB], _NEG)
                    if t + 1 < nsub:
                        sbuf[par, (t + 1) * SUB:, c0:c0 + SUB] = sc[SUB:]
                ts.append(f)
            return ts

        def sm_tasks(i, par):
            ts = []
            for j in range(BQ // RH):
                def f(j=j):
                    kvl = i * BQ + (j + 1) * RH
                    sc = sbuf[par, j * RH:(j + 1) * RH, 0:kvl]
                    m = jnp.max(sc, axis=1, keepdims=True)
                    p = jnp.exp2((sc - m) * scale)
                    ls[(i, j)] = jnp.sum(p, axis=1, keepdims=True)
                    pbuf[par, j * RH:(j + 1) * RH, 0:kvl] = p.astype(_BF16)
                ts.append(f)
            return ts

        def pv_tasks(i, par):
            ts = []
            for j in range(BQ // RH):
                def f(j=j):
                    kvl = i * BQ + (j + 1) * RH
                    o = _dot(pbuf[par, j * RH:(j + 1) * RH, 0:kvl], kv[slot, 0:kvl, D:2 * D])
                    cbuf[par, j * RH:(j + 1) * RH, :] = (o * (1.0 / ls[(i, j)])).astype(_BF16)
                ts.append(f)
            return ts

        def op_tasks(i, par):
            def f():
                r0, r1 = i * BQ, (i + 1) * BQ
                res = acc[:, r0:r1] + _dot_nt(wot[h], cbuf[par])
                if last:
                    stage[r0:r1, M:2 * M] = res.astype(_BF16).T
                    out_copy(i).start()
                else:
                    acc[:, r0:r1] = res
            return [f]

        kvt = [] if last else kv_proj_tasks(h + 1, 1 - slot)
        per = len(kvt) // NQ

        for f in s_tasks(order[0], 0):
            f()
        for n in range(NQ + 2):
            mx = s_tasks(order[n + 1], (n + 1) % 2) if n + 1 < NQ else []
            mx2 = []
            if 0 <= n - 2 < NQ:
                mx2 += op_tasks(order[n - 2], n % 2)
            if 0 <= n - 1 < NQ:
                mx2 += pv_tasks(order[n - 1], (n - 1) % 2)
            if n < NQ and not last:
                mx2 += kvt[n * per:(n + 1) * per]
            allm = []
            a = b = 0
            while a < len(mx) or b < len(mx2):
                if b >= len(mx2) or (a < len(mx) and a * len(mx2) <= b * len(mx)):
                    allm.append(mx[a])
                    a += 1
                else:
                    allm.append(mx2[b])
                    b += 1
            if n < NQ:
                _weave(sm_tasks(order[n], n % 2), allm)
            else:
                for f in allm:
                    f()

    def body(h, c):
        head(h, False)
        return c

    lax.fori_loop(0, H - 1, body, 0)
    head(H - 1, True)
    for i in range(NQ):
        out_copy(i).wait()


@jax.jit
def pallas_concat_heads__spectral_gfnet__compressed_kv_cla__prompt_kernel(
    A_x: jax.Array,
    A_w_r: jax.Array,
    A_w_i: jax.Array,
    B_x: jax.Array,
    B_c_kv: jax.Array,
    B_w_q: jax.Array,
    B_w_uk: jax.Array,
    B_w_uv: jax.Array,
    B_w_o: jax.Array,
):
    B, S, M = A_x.shape
    Df = M // 2 + 1
    C = B_c_kv.shape[-1]
    _, H, D = B_w_q.shape
    BQ = 512
    tables = [jnp.asarray(t) for t in _dft_tables(S, M)]

    vm = pltpu.VMEM
    HR = -(-Df // 8) * 8
    scratch = [
        vm((M, S), _BF16), vm((Df, S), _BF16), vm((Df, S), _BF16),
        vm((M, S), _BF16), vm((S, C), _BF16),
        vm((M, H, D), _BF16), vm((C, H, D), _BF16), vm((C, H, D), _BF16),
        vm((H, M, D), _BF16),
        vm((2 * HR, M), _BF16),
        vm((16, 256, 128), _BF16), vm((16, 256, 128), _BF16),
        vm((Df, M), _BF16), vm((Df, M), _BF16),
        vm((2 * HR, S), _F32), vm((S, Df), _F32), vm((S, Df), _F32),
        vm((16, S // 16, Df), _BF16), vm((16, S // 16, Df), _BF16),
        vm((S, M), _BF16),
        vm((H, M, D), _BF16), vm((H, C, 2 * D), _BF16),
        vm((H, S, D), _BF16), vm((2, S, 2 * D), _BF16),
        vm((M, S), _F32), vm((S, 2 * M), _BF16),
        vm((2, BQ, S), _F32), vm((2, BQ, S), _BF16), vm((2, BQ, D), _BF16),
        vm((5, S // 2, C // 2), _BF16),
        pltpu.SemaphoreType.DMA((16 + 2 * (C // 128),)),
        pltpu.SemaphoreType.DMA((S // BQ,)),
    ]
    any_spec = pl.BlockSpec(memory_space=pltpu.HBM)
    return pl.pallas_call(
        functools.partial(_kernel, S=S, M=M, H=H, D=D, C=C, BQ=BQ),
        in_specs=[any_spec] * 14 + [pl.BlockSpec(memory_space=pltpu.SMEM)],
        out_specs=any_spec,
        out_shape=jax.ShapeDtypeStruct((B, S, 2 * M), _BF16),
        scratch_shapes=scratch,
        compiler_params=pltpu.CompilerParams(vmem_limit_bytes=120 * 2**20),
        name="gfnet_cla",
    )(jnp.swapaxes(A_x, 1, 2), A_w_r.T, A_w_i.T, jnp.swapaxes(B_x, 1, 2), B_c_kv,
      B_w_q, B_w_uk, B_w_uv, jnp.swapaxes(B_w_o, 1, 2), *tables, jnp.asarray(np.zeros((1,), np.int32)))
```
